```python
import jax
import jax.numpy as jnp

def _softmax(x, axis=-1):
    return jax.nn.softmax(x, axis=axis)
def _gelu(x):
    return jax.nn.gelu(x, approximate=True)
def _silu(x):
    return jax.nn.silu(x)
def _sigmoid(x):
    return jax.nn.sigmoid(x)
def _layernorm(x, axis=-1, eps=1e-5):
    m = jnp.mean(x, axis=axis, keepdims=True)
    v = jnp.var(x, axis=axis, keepdims=True)
    return (x - m) / jnp.sqrt(v + eps)
def _scatter_add(tgt, idx, src, axis=0):
    return tgt.at[idx].add(src)
def _segment_sum(src, seg, n):
    return jax.ops.segment_sum(src, seg, n)
class _Rng:
    def __init__(self, key):
        self._k = key
    def _next(self):
        self._k, sub = jax.random.split(self._k)
        return sub
    def normal(self, shape):
        return jax.random.normal(self._next(), shape, dtype=jnp.bfloat16)
    def randint(self, lo, hi, shape):
        return jax.random.randint(self._next(), shape, lo, hi, dtype=jnp.int32)
    def uniform(self, shape, lo=0.0, hi=1.0):
        return jax.random.uniform(self._next(), shape, jnp.bfloat16, lo, hi)
    def permutation(self, n):
        return jax.random.permutation(self._next(), n)


kernel_name = 'recurrent_scan__sliding_local_dilated__swiglu_ffn__prompt'

def setup_inputs():
    _rng = _Rng(jax.random.key(int.from_bytes(__import__("os").urandom(4), "little")))
    _w = (lambda a: (lambda t: t.astype(jnp.bfloat16) if jnp.issubdtype(t.dtype, jnp.floating) else t)(jnp.asarray(a)))
    def _A_setup():
        B, S, D = 1, 2048, 1024
        return {
            "x": _w((lambda *s: _rng.normal(s) * 0.05)(B, S, D)),
            "wqkv": _w((lambda *s: _rng.normal(s) * 0.05)(D, 3 * D)),
            "wo": _w((lambda *s: _rng.normal(s) * 0.05)(D, D)),
        }
    _A_in = _A_setup()

    def _B_setup():
        B, S, D, F = 1, 2048, 1024, 3584
        return {
            "x": _w((lambda *s: _rng.normal(s) * 0.05)(B, S, D)),
            "w_gate": _w((lambda *s: _rng.normal(s) * 0.05)(D, F)),
            "w_up": _w((lambda *s: _rng.normal(s) * 0.05)(D, F)),
            "w_down": _w((lambda *s: _rng.normal(s) * 0.05)(F, D)),
        }
    _B_in = _B_setup()

    return {
        "A_x": _A_in["x"],
        "A_wqkv": _A_in["wqkv"],
        "A_wo": _A_in["wo"],
        "B_x": _B_in["x"],
        "B_w_gate": _B_in["w_gate"],
        "B_w_up": _B_in["w_up"],
        "B_w_down": _B_in["w_down"],
    }

def reference(A_x, A_wqkv, A_wo, B_x, B_w_gate, B_w_up, B_w_down):
    def _A_ref(x, wqkv, wo):
        B, S, D = x.shape
        H = 32; Dh = D // H
        W, dil = 8, 2
        qkv = (lambda x, *d: x.transpose(*d))((x @ wqkv).reshape(B, S, 3, H, Dh), 2, 0, 3, 1, 4)
        q, k, v = qkv[0], qkv[1], qkv[2]
        scale = Dh ** -0.5
        pos = jnp.arange(S)
        off = jnp.arange(W) * dil
        idx = pos[:, None] - off[None, :]
        mask = idx >= 0
        idx_c = jnp.where(mask, idx, 0).reshape(-1)
        kg = k[:, :, idx_c, :].reshape(B, H, S, W, Dh)
        vg = v[:, :, idx_c, :].reshape(B, H, S, W, Dh)
        logits = jnp.einsum("bhsd,bhswd->bhsw", q, kg) * scale
        logits = jnp.where(mask[None, None, :, :], logits, -1e9)
        attn = _softmax(logits, axis=-1)
        o = jnp.einsum("bhsw,bhswd->bhsd", attn, vg)
        return (lambda x, *d: x.transpose(*d))(o, 0, 2, 1, 3).reshape(B, S, D) @ wo

    def _B_ref(x, w_gate, w_up, w_down):
        g = _silu(x @ w_gate)
        u = x @ w_up
        return (g * u) @ w_down

    x = A_x
    xn = _layernorm(x, axis=-1)
    s = _A_ref(xn, A_wqkv, A_wo)
    g = _silu(_B_ref(xn, B_w_gate, B_w_up, B_w_down))
    return x + s * g
```

```python
import contextlib
import functools
import numpy as np
import jax
import jax.numpy as jnp
import jax.experimental.pallas as pl
import jax.experimental.pallas.tpu as pltpu
from jax import lax

S, D, F = 2048, 1024, 3584
H, DH, W, DIL = 32, 32, 8, 2
HALO = 16
LOG2E = 1.4426950408889634
NT = D // 128


def _sigmoid(x):
    return pltpu.reciprocal(1.0 + jnp.exp2(x * (-LOG2E)), approx=True)


def _swap_heads(xs):
    shape = xs[0].shape
    lane = lax.broadcasted_iota(jnp.int32, shape, 1)
    g = lane >> 4
    e = lane & 15
    zs = []
    for s in range(8):
        t = (g - s) & 7
        idx = (e & 3) * 32 + t * 4 + (e >> 2)
        zs.append(jnp.take_along_axis(xs[s], idx, axis=1, mode="promise_in_bounds"))
    a = [zs[(-t) % 8] for t in range(8)]
    for b in range(3):
        bit = ((g >> b) & 1) == 1
        a = [jnp.where(bit, a[(t - (1 << b)) % 8], a[t]) for t in range(8)]
    j = lane >> 5
    sm = (lane >> 2) & 7
    hh = lane & 3
    out = []
    for t in range(8):
        idx = ((sm + t) & 7) * 16 + j * 4 + hh
        out.append(jnp.take_along_axis(a[t], idx, axis=1, mode="promise_in_bounds"))
    return out


def make(BM=256, BF=512, QM=512, RB=64, PR=128, scopes=False, apos=0, pin=2, ffn_at=1, dorder=0):
    NSTEP = S // BM
    NF = F // BF
    NQM = S // QM
    KC = D // NQM

    def scope(name):
        return jax.named_scope(name) if scopes else contextlib.nullcontext()

    def kernel(x_h, wqkv_h, wo_h, wg_h, wu_h, wd_h, out_h,
               x_v, xn_v, wqkv_v, wp_v, wo_v, wg_v, wu_v, wd_v, qkv_s, out_v, sem_x, sem_q, sem_w, sem_out):
        def x_copy(r):
            return pltpu.make_async_copy(x_h.at[pl.ds(r * QM, QM), :], x_v.at[pl.ds(r * QM, QM), :], sem_x.at[r])
        def q_copy(m, r):
            return pltpu.make_async_copy(wqkv_h.at[pl.ds(r * KC, KC), pl.ds(m * D, D)],
                                         wqkv_v.at[m, pl.ds(r * KC, KC), :], sem_q.at[m * NQM + r])
        w_copies = [pltpu.make_async_copy(wg_h, wg_v, sem_w.at[0]),
                    pltpu.make_async_copy(wu_h, wu_v, sem_w.at[1]),
                    pltpu.make_async_copy(wd_h, wd_v, sem_w.at[2]),
                    pltpu.make_async_copy(wo_h, wo_v, sem_w.at[3])]
        def out_copy(i):
            return pltpu.make_async_copy(out_v.at[pl.ds(i * BM, BM), :], out_h.at[pl.ds(i * BM, BM), :], sem_out.at[i])

        def permute_rows(ms, md, k0):
            for p0 in range(0, KC, 2 * PR):
                src = wqkv_v[ms, pl.ds(pl.multiple_of(k0 + p0, 2 * PR), 2 * PR), :]
                u = pltpu.bitcast(src, jnp.uint32)
                ys = _swap_heads([u[:, s * 128:(s + 1) * 128] for s in range(NT)])
                dst0 = pl.multiple_of((k0 + p0) // 2, PR)
                for t in range(NT):
                    wp_v[md, pl.ds(dst0, PR), t * 128:(t + 1) * 128] = ys[t]

        def layernorm(src0, dst0):
            x = x_v[pl.ds(src0, QM), :].astype(jnp.float32)
            m = jnp.mean(x, axis=-1, keepdims=True)
            xc = x - m
            var = jnp.mean(xc * xc, axis=-1, keepdims=True)
            xn_v[pl.ds(dst0, QM), :] = (xc * lax.rsqrt(var + 1e-5)).astype(jnp.bfloat16)

        def project(m, r0):
            wmat = pltpu.bitcast(wp_v[m], jnp.bfloat16)
            res = jnp.dot(xn_v[pl.ds(r0, QM), :], wmat, preferred_element_type=jnp.float32)
            for t in range(NT):
                qkv_s[m * NT + t, pl.ds(r0 + HALO, QM), :] = res[:, t * 128:(t + 1) * 128]

        if dorder == 0:
            x_copy(0).start()
            for r in range(NQM):
                q_copy(0, r).start()
        else:
            for r in range(NQM):
                q_copy(0, r).start()
            x_copy(0).start()
        qkv_s[NT:3 * NT, 0:HALO, :] = jnp.zeros((2 * NT, HALO, 128), jnp.float32)

        def pq_body(r, _):
            with scope("wwq"):
                q_copy(0, r).wait()
            permute_rows(0, 0, r * KC)
            return 0
        if dorder == 0:
            with scope("ln0"):
                x_copy(0).wait()
                x_copy(1).start()
                q_copy(1, 0).start()
                layernorm(0, 0)
            with scope("permq"):
                lax.fori_loop(0, NQM, pq_body, 0)
        else:
            with scope("permq"):
                lax.fori_loop(0, NQM, pq_body, 0)
            with scope("ln0"):
                x_copy(1).start()
                q_copy(1, 0).start()
                x_copy(0).wait()
                layernorm(0, 0)
        for r in range(2, NQM):
            x_copy(r).start()
        for r in range(1, NQM):
            q_copy(1, r).start()

        def q_body(r, _):
            @pl.when(r == 1)
            def _():
                for r2 in range(NQM):
                    q_copy(2, r2).start()
            @pl.when(r + 1 < NQM)
            def _():
                with scope("wx"):
                    x_copy(r + 1).wait()
            with scope("wwk"):
                q_copy(1, r).wait()
            r0 = pl.multiple_of(r * QM, QM)
            project(0, r0)
            layernorm(pl.multiple_of(jnp.minimum(r + 1, NQM - 1) * QM, QM), pl.multiple_of(r0 + QM, QM))
            permute_rows(1, 1, r * KC)
            return 0
        with scope("q"):
            lax.fori_loop(0, NQM, q_body, 0)

        def kv_body(it, _):
            m = 1 + it // NQM
            r = it % NQM
            @pl.when(it == ffn_at)
            def _():
                for cp in w_copies:
                    cp.start()
            @pl.when(m < 2)
            def _():
                with scope("wwv"):
                    q_copy(2, r).wait()
            project(m, pl.multiple_of(r * QM, QM))
            permute_rows(2, m + 1, r * KC)
            return 0
        with scope("kv"):
            lax.fori_loop(0, 2 * NQM, kv_body, 0)

        with scope("wwait"):
            for cp in w_copies:
                cp.wait()

        def main_body(i, _):
            base = pl.multiple_of(i * BM, BM)
            rows = pl.ds(base, BM)

            def attn_rows(r0):
                b0 = base + (HALO + r0)
                q = [qkv_s[t, pl.ds(b0, RB), :] * (DH ** -0.5 * LOG2E) for t in range(NT)]
                lg = []
                for w in range(W):
                    p = None
                    for t in range(NT):
                        pr = q[t] * qkv_s[NT + t, pl.ds(b0 - DIL * w, RB), :]
                        p = pr if p is None else p + pr
                    p = p + pltpu.roll(p, 64, 1)
                    p = p + pltpu.roll(p, 32, 1)
                    if w > 0 and r0 < HALO:
                        row_top = lax.broadcasted_iota(jnp.int32, (HALO, 128), 0) + base
                        top = jnp.where(row_top >= DIL * w, p[:HALO], -1e9)
                        p = jnp.concatenate([top, p[HALO:]], axis=0) if RB > HALO else top
                    lg.append(p)
                mx = functools.reduce(jnp.maximum, lg)
                e = [jnp.exp2(l - mx) for l in lg]
                den = functools.reduce(lambda a, b: a + b, e)
                rinv = pltpu.reciprocal(den, approx=True)
                e = [ew * rinv for ew in e]
                os_ = []
                for t in range(NT):
                    o = None
                    for w in range(W):
                        ov = e[w] * qkv_s[2 * NT + t, pl.ds(b0 - DIL * w, RB), :]
                        o = ov if o is None else o + ov
                    os_.append(pltpu.bitcast(o.astype(jnp.bfloat16), jnp.uint32))
                os_ = _swap_heads(os_)
                return pltpu.bitcast(jnp.concatenate(os_, axis=1), jnp.bfloat16)

            xn = xn_v[rows, :]
            acc = None
            pieces = list(range(0, BM, RB))
            outs = [None] * len(pieces)
            ss = [None] * len(pieces)
            slot = {c: [] for c in range(NF)}
            for n in range(len(pieces)):
                slot[min(apos + n * (NF - apos) // len(pieces), NF - 1)].append(n)
            for c in range(NF):
                cs = slice(c * BF, (c + 1) * BF)
                g = jnp.dot(xn, wg_v[:, cs], preferred_element_type=jnp.float32)
                u = jnp.dot(xn, wu_v[:, cs], preferred_element_type=jnp.float32)
                for n in slot[c]:
                    outs[n] = attn_rows(pieces[n])
                    if pin == 2:
                        ss[n] = jnp.dot(outs[n], wo_v[...], preferred_element_type=jnp.float32)
                h = (g * _sigmoid(g) * u).astype(jnp.bfloat16)
                d = jnp.dot(h, wd_v[cs, :], preferred_element_type=jnp.float32)
                acc = d if acc is None else acc + d
            if pin == 2:
                s = jnp.concatenate(ss, axis=0) if len(ss) > 1 else ss[0]
            else:
                o = jnp.concatenate(outs, axis=0) if len(outs) > 1 else outs[0]
                s = jnp.dot(o, wo_v[...], preferred_element_type=jnp.float32)
            gy = acc * _sigmoid(acc)
            out_v[rows, :] = (x_v[rows, :].astype(jnp.float32) + s * gy).astype(out_v.dtype)
            out_copy(i).start()
            return 0
        with scope("main"):
            lax.fori_loop(0, NSTEP, main_body, 0)
        for i in range(NSTEP):
            out_copy(i).wait()

    def fn(A_x, A_wqkv, A_wo, B_x, B_w_gate, B_w_up, B_w_down):
        x = A_x.reshape(S, D)
        any_spec = pl.BlockSpec(memory_space=pl.ANY)
        out = pl.pallas_call(
            kernel,
            in_specs=[any_spec] * 6,
            out_specs=any_spec,
            out_shape=jax.ShapeDtypeStruct((S, D), jnp.bfloat16),
            scratch_shapes=[
                pltpu.VMEM((S, D), jnp.bfloat16),
                pltpu.VMEM((S + QM, D), jnp.bfloat16),
                pltpu.VMEM((3, D, D), jnp.bfloat16),
                pltpu.VMEM((4, D // 2, D), jnp.uint32),
                pltpu.VMEM((D, D), jnp.bfloat16),
                pltpu.VMEM((D, F), jnp.bfloat16),
                pltpu.VMEM((D, F), jnp.bfloat16),
                pltpu.VMEM((F, D), jnp.bfloat16),
                pltpu.VMEM((3 * NT, HALO + S, 128), jnp.float32),
                pltpu.VMEM((S, D), jnp.bfloat16),
                pltpu.SemaphoreType.DMA((NQM,)),
                pltpu.SemaphoreType.DMA((3 * NQM,)),
                pltpu.SemaphoreType.DMA((4,)),
                pltpu.SemaphoreType.DMA((NSTEP,)),
            ],
            compiler_params=pltpu.CompilerParams(vmem_limit_bytes=120 * 1024 * 1024),
        )(x, A_wqkv, A_wo, B_w_gate, B_w_up, B_w_down)
        return out.reshape(1, S, D)
    return fn


@jax.jit
def pallas_recurrent_scan__sliding_local_dilated__swiglu_ffn__prompt_kernel(
    A_x: jax.Array,
    A_wqkv: jax.Array,
    A_wo: jax.Array,
    B_x: jax.Array,
    B_w_gate: jax.Array,
    B_w_up: jax.Array,
    B_w_down: jax.Array,
):
    return make(dorder=1)(A_x, A_wqkv, A_wo, B_x, B_w_gate, B_w_up, B_w_down)
```

```python
import contextlib
import functools
import numpy as np
import jax
import jax.numpy as jnp
import jax.experimental.pallas as pl
import jax.experimental.pallas.tpu as pltpu
from jax import lax

S, D, F = 2048, 1024, 3584
H, DH, W, DIL = 32, 32, 8, 2
HALO = 16
LOG2E = 1.4426950408889634
NT = D // 128


def _sigmoid(x):
    return pltpu.reciprocal(1.0 + jnp.exp2(x * (-LOG2E)), approx=True)


def _swap_heads(xs):
    shape = xs[0].shape
    lane = lax.broadcasted_iota(jnp.int32, shape, 1)
    g = lane >> 4
    e = lane & 15
    zs = []
    for s in range(8):
        t = (g - s) & 7
        idx = (e & 3) * 32 + t * 4 + (e >> 2)
        zs.append(jnp.take_along_axis(xs[s], idx, axis=1, mode="promise_in_bounds"))
    a = [zs[(-t) % 8] for t in range(8)]
    for b in range(3):
        bit = ((g >> b) & 1) == 1
        a = [jnp.where(bit, a[(t - (1 << b)) % 8], a[t]) for t in range(8)]
    j = lane >> 5
    sm = (lane >> 2) & 7
    hh = lane & 3
    out = []
    for t in range(8):
        idx = ((sm + t) & 7) * 16 + j * 4 + hh
        out.append(jnp.take_along_axis(a[t], idx, axis=1, mode="promise_in_bounds"))
    return out


def make(BM=256, BF=512, QM=512, RB=64, PR=128, scopes=False, apos=0, pin=2, ffn_at=1, LNR=16, QPR=64, flags=None, aord=0, npin=14):
    NSTEP = S // BM
    NF = F // BF
    NQM = S // QM
    QP = S // (2 * NQM)
    KC = D // NQM

    def scope(name):
        return jax.named_scope(name) if scopes else contextlib.nullcontext()

    def kernel(x_h, wqkv_h, wo_h, wg_h, wu_h, wd_h, out_h,
               x_v, xn_v, wqkv_v, wp_v, wo_v, wg_v, wu_v, wd_v, kv_s, q_s, st_s, cs_s, out_v, flag_s, sem_x, sem_q, sem_w, sem_out):
        def x_copy(r):
            return pltpu.make_async_copy(x_h.at[pl.ds(r * QM, QM), :], x_v.at[pl.ds(r * QM, QM), :], sem_x.at[r])
        def q_copy(m, r):
            return pltpu.make_async_copy(wqkv_h.at[pl.ds(r * KC, KC), pl.ds(m * D, D)],
                                         wqkv_v.at[m, pl.ds(r * KC, KC), :], sem_q.at[m * NQM + r])
        wq_copy = pltpu.make_async_copy(wqkv_h.at[:, pl.ds(0, D)], wqkv_v.at[0], sem_q.at[0])
        w_copies = [pltpu.make_async_copy(wg_h, wg_v, sem_w.at[0]),
                    pltpu.make_async_copy(wu_h, wu_v, sem_w.at[1]),
                    pltpu.make_async_copy(wd_h, wd_v, sem_w.at[2]),
                    pltpu.make_async_copy(wo_h, wo_v, sem_w.at[3])]
        def out_copy(i):
            return pltpu.make_async_copy(out_v.at[pl.ds(i * BM, BM), :], out_h.at[pl.ds(i * BM, BM), :], sem_out.at[i])

        def permute_rows(ms, md, k0):
            for p0 in range(0, KC, 2 * PR):
                src = wqkv_v[ms, pl.ds(pl.multiple_of(k0 + p0, 2 * PR), 2 * PR), :]
                u = pltpu.bitcast(src, jnp.uint32)
                ys = _swap_heads([u[:, s * 128:(s + 1) * 128] for s in range(NT)])
                dst0 = pl.multiple_of((k0 + p0) // 2, PR)
                for t in range(NT):
                    wp_v[md, pl.ds(dst0, PR), t * 128:(t + 1) * 128] = ys[t]

        def project(m, r0):
            wmat = pltpu.bitcast(wp_v[m], jnp.bfloat16)
            xn = pltpu.bitcast(xn_v[pl.ds(pl.multiple_of(r0 // 2, QM // 2), QM // 2), :], jnp.bfloat16)
            res = jnp.dot(xn, wmat, preferred_element_type=jnp.float32)
            for t in range(NT):
                kv_s[(m - 1) * NT + t, pl.ds(r0 + HALO, QM), :] = res[:, t * 128:(t + 1) * 128]

        flag_s[0] = 1
        x_copy(0).start()
        wq_copy.start()
        q_copy(1, 0).start()
        kv_s[:, 0:HALO, :] = jnp.zeros((2 * NT, HALO, 128), jnp.float32)

        def q_body(r, _):
            with scope("wx"):
                x_copy(r).wait()
            with scope("wwk"):
                q_copy(1, r).wait()
            @pl.when(r == 0)
            def _():
                with scope("wwq"):
                    wq_copy.wait()
                for r2 in range(1, NQM):
                    x_copy(r2).start()
                    q_copy(1, r2).start()
            @pl.when(r == 1)
            def _():
                for r2 in range(NQM):
                    q_copy(2, r2).start()
            r0 = pl.multiple_of(r * QM, QM)
            res = jnp.dot(x_v[pl.ds(r0, QM), :], wqkv_v[0], preferred_element_type=jnp.float32)
            for t in range(NT):
                q_s[t, pl.ds(r0, QM), :] = res[:, t * 128:(t + 1) * 128]
            CW = D // NQM
            ccols = pl.ds(pl.multiple_of(r * CW, CW), CW)
            cs = jnp.sum(wqkv_v[0, :, ccols].astype(jnp.float32), axis=0, keepdims=True)
            cs_s[:, ccols] = jnp.broadcast_to(cs, (8, CW))
            for c0 in range(0, QM, LNR):
                rws = pl.ds(r0 + c0, LNR)
                x = x_v[rws, :].astype(jnp.float32)
                mu = jnp.mean(x, axis=-1, keepdims=True)
                xc = x - mu
                var = jnp.mean(xc * xc, axis=-1, keepdims=True)
                rs = lax.rsqrt(var + 1e-5)
                xn_v[pl.ds(pl.multiple_of((r0 + c0) // 2, LNR // 2), LNR // 2), :] = pltpu.bitcast(
                    (xc * rs).astype(jnp.bfloat16), jnp.uint32)
                st_s[0, rws, :] = jnp.broadcast_to(mu, (LNR, 128))
                st_s[1, rws, :] = jnp.broadcast_to(rs * (DH ** -0.5 * LOG2E), (LNR, 128))
            permute_rows(1, 1, r * KC)
            return 0
        with scope("q"):
            lax.fori_loop(0, NQM, q_body, 0)

        def kv_body(it, _):
            m = 1 + it // NQM
            r = it % NQM
            @pl.when(it == ffn_at)
            def _():
                for cp in w_copies:
                    cp.start()
            @pl.when(m < 2)
            def _():
                with scope("wwv"):
                    q_copy(2, r).wait()
            project(m, pl.multiple_of(r * QM, QM))
            permute_rows(2, m + 1, r * KC)
            for p0 in range(0, QP, QPR):
                rws = pl.ds(pl.multiple_of(it * QP + p0, QPR), QPR)
                mu = st_s[0, rws, :]
                rs = st_s[1, rws, :]
                us = []
                for t in range(NT):
                    cst = jnp.broadcast_to(cs_s[0:1, t * 128:(t + 1) * 128], (QPR, 128))
                    qn = (q_s[t, rws, :] - mu * cst) * rs
                    us.append(pltpu.bitcast(qn.astype(jnp.bfloat16), jnp.uint32))
                ys = _swap_heads(us)
                for t in range(NT):
                    q_s[t, rws, :] = pltpu.bitcast(ys[t], jnp.bfloat16).astype(jnp.float32)
            return 0
        with scope("kv"):
            lax.fori_loop(0, 2 * NQM, kv_body, 0)

        with scope("wwait"):
            for cp in w_copies:
                cp.wait()

        def main_body(i, _):
            base = pl.multiple_of(i * BM, BM)
            rows = pl.ds(base, BM)

            def attn_rows(r0):
                b0 = base + (HALO + r0)
                q = [q_s[t, pl.ds(base + r0, RB), :] for t in range(NT)]
                lg = []
                for w in range(W):
                    p = None
                    for t in range(NT):
                        pr = q[t] * kv_s[t, pl.ds(b0 - DIL * w, RB), :]
                        p = pr if p is None else p + pr
                    p = p + pltpu.roll(p, 64, 1)
                    p = p + pltpu.roll(p, 32, 1)
                    if w > 0 and r0 < HALO:
                        row_top = lax.broadcasted_iota(jnp.int32, (HALO, 128), 0) + base
                        top = jnp.where(row_top >= DIL * w, p[:HALO], -1e9)
                        p = jnp.concatenate([top, p[HALO:]], axis=0) if RB > HALO else top
                    lg.append(p)
                mx = functools.reduce(jnp.maximum, lg)
                e = [jnp.exp2(l - mx) for l in lg]
                den = functools.reduce(lambda a, b: a + b, e)
                rinv = pltpu.reciprocal(den, approx=True)
                e = [ew * rinv for ew in e]
                os_ = []
                for t in range(NT):
                    o = None
                    for w in range(W):
                        ov = e[w] * kv_s[NT + t, pl.ds(b0 - DIL * w, RB), :]
                        o = ov if o is None else o + ov
                    os_.append(pltpu.bitcast(o.astype(jnp.bfloat16), jnp.uint32))
                os_ = _swap_heads(os_)
                return jnp.concatenate(os_, axis=1)

            xu = xn_v[pl.ds(pl.multiple_of(base // 2, BM // 2), BM // 2), :]
            xn = pltpu.bitcast(xu, jnp.bfloat16)
            acc = None
            pieces = list(range(0, BM, RB))
            outs = [None] * len(pieces)
            ss = [None] * len(pieces)
            if pin == 3:
                keep = flag_s[0] > 0
                for n in range(len(pieces)):
                    outs[n] = attn_rows(pieces[n])
                at = {}
                for n in range(len(pieces)):
                    at.setdefault(apos + n * (npin - apos) // len(pieces), []).append(n)
                def pinned(pos):
                    if pos not in at:
                        return xn
                    head = xu[0:8, 0:128]
                    for n in at[pos]:
                        head = jnp.where(keep, head, outs[n][0:8, 0:128])
                    top = jnp.concatenate([head, xu[0:8, 128:]], axis=1)
                    return pltpu.bitcast(jnp.concatenate([top, xu[8:]], axis=0), jnp.bfloat16)
                for c in range(NF):
                    cs = slice(c * BF, (c + 1) * BF)
                    g = jnp.dot(pinned(2 * c), wg_v[:, cs], preferred_element_type=jnp.float32)
                    u = jnp.dot(pinned(2 * c + 1), wu_v[:, cs], preferred_element_type=jnp.float32)
                    h = (g * _sigmoid(g) * u).astype(jnp.bfloat16)
                    d = jnp.dot(h, wd_v[cs, :], preferred_element_type=jnp.float32)
                    acc = d if acc is None else acc + d
                o = pltpu.bitcast(jnp.concatenate(outs, axis=0), jnp.bfloat16)
                s = jnp.dot(o, wo_v[...], preferred_element_type=jnp.float32)
            else:
                slot = {c: [] for c in range(NF)}
                for n in range(len(pieces)):
                    slot[min(apos + n * (NF - apos) // len(pieces), NF - 1)].append(n)
                for c in range(NF):
                    cs = slice(c * BF, (c + 1) * BF)
                    g = jnp.dot(xn, wg_v[:, cs], preferred_element_type=jnp.float32)
                    u = jnp.dot(xn, wu_v[:, cs], preferred_element_type=jnp.float32)
                    for n in slot[c]:
                        outs[n] = pltpu.bitcast(attn_rows(pieces[n]), jnp.bfloat16)
                        if pin == 2:
                            ss[n] = jnp.dot(outs[n], wo_v[...], preferred_element_type=jnp.float32)
                    h = (g * _sigmoid(g) * u).astype(jnp.bfloat16)
                    d = jnp.dot(h, wd_v[cs, :], preferred_element_type=jnp.float32)
                    acc = d if acc is None else acc + d
                if pin == 2:
                    s = jnp.concatenate(ss, axis=0) if len(ss) > 1 else ss[0]
                else:
                    o = jnp.concatenate(outs, axis=0) if len(outs) > 1 else outs[0]
                    s = jnp.dot(o, wo_v[...], preferred_element_type=jnp.float32)
            gy = acc * _sigmoid(acc)
            out_v[rows, :] = (x_v[rows, :].astype(jnp.float32) + s * gy).astype(out_v.dtype)
            out_copy(i).start()
            return 0
        with scope("main"):
            lax.fori_loop(0, NSTEP, main_body, 0)
        for i in range(NSTEP):
            out_copy(i).wait()

    def fn(A_x, A_wqkv, A_wo, B_x, B_w_gate, B_w_up, B_w_down):
        x = A_x.reshape(S, D)
        any_spec = pl.BlockSpec(memory_space=pl.ANY)
        out = pl.pallas_call(
            kernel,
            in_specs=[any_spec] * 6,
            out_specs=any_spec,
            out_shape=jax.ShapeDtypeStruct((S, D), jnp.bfloat16),
            scratch_shapes=[
                pltpu.VMEM((S, D), jnp.bfloat16),
                pltpu.VMEM((S // 2, D), jnp.uint32),
                pltpu.VMEM((3, D, D), jnp.bfloat16),
                pltpu.VMEM((4, D // 2, D), jnp.uint32),
                pltpu.VMEM((D, D), jnp.bfloat16),
                pltpu.VMEM((D, F), jnp.bfloat16),
                pltpu.VMEM((D, F), jnp.bfloat16),
                pltpu.VMEM((F, D), jnp.bfloat16),
                pltpu.VMEM((2 * NT, HALO + S, 128), jnp.float32),
                pltpu.VMEM((NT, S, 128), jnp.float32),
                pltpu.VMEM((2, S, 128), jnp.float32),
                pltpu.VMEM((8, D), jnp.float32),
                pltpu.VMEM((S, D), jnp.bfloat16),
                pltpu.SMEM((1,), jnp.int32),
                pltpu.SemaphoreType.DMA((NQM,)),
                pltpu.SemaphoreType.DMA((3 * NQM,)),
                pltpu.SemaphoreType.DMA((4,)),
                pltpu.SemaphoreType.DMA((NSTEP,)),
            ],
            compiler_params=pltpu.CompilerParams(vmem_limit_bytes=120 * 1024 * 1024, flags=flags),
        )(x, A_wqkv, A_wo, B_w_gate, B_w_up, B_w_down)
        return out.reshape(1, S, D)
    return fn


@jax.jit
def pallas_recurrent_scan__sliding_local_dilated__swiglu_ffn__prompt_kernel(
    A_x: jax.Array,
    A_wqkv: jax.Array,
    A_wo: jax.Array,
    B_x: jax.Array,
    B_w_gate: jax.Array,
    B_w_up: jax.Array,
    B_w_down: jax.Array,
):
    return make(pin=3, RB=16, apos=1)(A_x, A_wqkv, A_wo, B_x, B_w_gate, B_w_up, B_w_down)
```

```python
import contextlib
import functools
import numpy as np
import jax
import jax.numpy as jnp
import jax.experimental.pallas as pl
import jax.experimental.pallas.tpu as pltpu
from jax import lax

S, D, F = 2048, 1024, 3584
H, DH, W, DIL = 32, 32, 8, 2
HALO = 16
LOG2E = 1.4426950408889634
NT = D // 128
QSCALE = DH ** -0.5 * LOG2E


def _sigmoid(x):
    return pltpu.reciprocal(1.0 + jnp.exp2(x * (-LOG2E)), approx=True)


def _swap_heads(xs):
    shape = xs[0].shape
    lane = lax.broadcasted_iota(jnp.int32, shape, 1)
    g = lane >> 4
    e = lane & 15
    zs = []
    for s in range(8):
        t = (g - s) & 7
        idx = (e & 3) * 32 + t * 4 + (e >> 2)
        zs.append(jnp.take_along_axis(xs[s], idx, axis=1, mode="promise_in_bounds"))
    a = [zs[(-t) % 8] for t in range(8)]
    for b in range(3):
        bit = ((g >> b) & 1) == 1
        a = [jnp.where(bit, a[(t - (1 << b)) % 8], a[t]) for t in range(8)]
    j = lane >> 5
    sm = (lane >> 2) & 7
    hh = lane & 3
    out = []
    for t in range(8):
        idx = ((sm + t) & 7) * 16 + j * 4 + hh
        out.append(jnp.take_along_axis(a[t], idx, axis=1, mode="promise_in_bounds"))
    return out


def make(BM=256, BF=512, QM=512, RB=16, PR=128, scopes=False, apos=1, npin=14, ffn_at=1, LNR=16, QPR=64,
         QSUB=128, lnpin=True, first=(384, 640), nosem=False, nobounds=False):
    NSTEP = S // BM
    NF = F // BF
    NQM = S // QM
    QP = S // (2 * NQM)
    KC = D // NQM
    WQ0 = S

    def scope(name):
        return jax.named_scope(name) if scopes else contextlib.nullcontext()

    def kernel(x_h, wqkv_h, wo_h, wg_h, wu_h, wd_h, out_h,
               in_v, xn_v, wp_v, wo_v, wg_v, wu_v, wd_v, kv_s, q_s, st_s, cs_s, out_v, flag_s,
               sem_x, sem_q, sem_kv, sem_w, sem_out):
        def x_copy(r):
            return pltpu.make_async_copy(x_h.at[pl.ds(r * QM, QM), :], in_v.at[pl.ds(r * QM, QM), :], sem_x.at[r])
        def wq_copy(i):
            c0 = sum(first[:i])
            return pltpu.make_async_copy(wqkv_h.at[:, pl.ds(c0, first[i])],
                                         in_v.at[pl.ds(WQ0, D), pl.ds(c0, first[i])], sem_q.at[i])
        def wkv_copy(m, r):
            return pltpu.make_async_copy(wqkv_h.at[pl.ds(r * KC, KC), pl.ds(m * D, D)],
                                         in_v.at[pl.ds(WQ0 + m * D + r * KC, KC), :], sem_kv.at[(m - 1) * NQM + r])
        w_copies = [pltpu.make_async_copy(wg_h, wg_v, sem_w.at[0]),
                    pltpu.make_async_copy(wu_h, wu_v, sem_w.at[1]),
                    pltpu.make_async_copy(wd_h, wd_v, sem_w.at[2]),
                    pltpu.make_async_copy(wo_h, wo_v, sem_w.at[3])]
        def out_copy(i):
            return pltpu.make_async_copy(out_v.at[pl.ds(i * BM, BM), :], out_h.at[pl.ds(i * BM, BM), :], sem_out.at[i])

        def permute_rows(ms, md, k0):
            for p0 in range(0, KC, 2 * PR):
                src = in_v[pl.ds(pl.multiple_of(WQ0 + ms * D + k0 + p0, 2 * PR), 2 * PR), :]
                u = pltpu.bitcast(src, jnp.uint32)
                ys = _swap_heads([u[:, s * 128:(s + 1) * 128] for s in range(NT)])
                dst0 = pl.multiple_of((k0 + p0) // 2, PR)
                for t in range(NT):
                    wp_v[md, pl.ds(dst0, PR), t * 128:(t + 1) * 128] = ys[t]

        def layernorm_piece(r0):
            rws = pl.ds(pl.multiple_of(r0, LNR), LNR)
            x = in_v[rws, :].astype(jnp.float32)
            mu = jnp.mean(x, axis=-1, keepdims=True)
            xc = x - mu
            var = jnp.mean(xc * xc, axis=-1, keepdims=True)
            rs = lax.rsqrt(var + 1e-5)
            xn = pltpu.bitcast((xc * rs).astype(jnp.bfloat16), jnp.uint32)
            xn_v[pl.ds(pl.multiple_of(r0 // 2, LNR // 2), LNR // 2), :] = xn
            st_s[0, rws, :] = jnp.broadcast_to(mu, (LNR, 128))
            st_s[1, rws, :] = jnp.broadcast_to(rs * QSCALE, (LNR, 128))
            return xn

        def q_store(res, r0, c0):
            for j in range(res.shape[1] // 128):
                q_s[c0 // 128 + j, pl.ds(r0, QM), :] = res[:, j * 128:(j + 1) * 128]

        x_copy(0).start()
        for i in range(len(first)):
            wq_copy(i).start()
        wkv_copy(1, 0).start()
        for r in range(1, NQM):
            x_copy(r).start()
            wkv_copy(1, r).start()
        for r in range(NQM):
            wkv_copy(2, r).start()
        flag_s[0] = 1
        kv_s[:, 0:HALO, :] = jnp.zeros((2 * NT, HALO, 128), jnp.float32)

        def q_body(r, _):
            r0 = pl.multiple_of(r * QM, QM)
            npc = QM // LNR
            keep = flag_s[0] > 0
            nseg = len(first)
            nsub_tot = D // QSUB
            sub = 0
            for i in range(nseg):
                with scope("wq%d" % i):
                    if i == 0:
                        x_copy(r).wait()
                    if i == nseg - 1:
                        wkv_copy(1, r).wait()
                    @pl.when(r == 0)
                    def _():
                        wq_copy(i).wait()
                if i == nseg - 1:
                    @pl.when(r == ffn_at)
                    def _():
                        for cp in w_copies:
                            cp.start()
                xb = in_v[pl.ds(r0, QM), :]
                c0, cw = sum(first[:i]), first[i]
                nsub = cw // QSUB
                mine = [n for n in range(npc) if c0 <= n * D // npc < c0 + cw]
                xns = {n: layernorm_piece(r0 + n * LNR) for n in mine}
                for j in range(nsub):
                    lhs = xb
                    tied = [n for k, n in enumerate(mine) if lnpin and 1 + k * (nsub - 1) // len(mine) == j]
                    if tied:
                        head = pltpu.bitcast(xb[0:16, 0:128], jnp.uint32)
                        for n in tied:
                            head = jnp.where(keep, head, xns[n][0:8, 0:128])
                        top = jnp.concatenate([pltpu.bitcast(head, jnp.bfloat16), xb[0:16, 128:]], axis=1)
                        lhs = jnp.concatenate([top, xb[16:]], axis=0)
                    cols = slice(c0 + j * QSUB, c0 + (j + 1) * QSUB)
                    q_store(jnp.dot(lhs, in_v[WQ0:WQ0 + D, cols], preferred_element_type=jnp.float32), r0, cols.start)
                if i == nseg - 1:
                    CW = D // NQM
                    ccols = pl.ds(pl.multiple_of(r * CW, CW), CW)
                    cs = jnp.sum(in_v[WQ0:WQ0 + D, ccols].astype(jnp.float32), axis=0, keepdims=True)
                    cs_s[:, ccols] = jnp.broadcast_to(cs, (8, CW))
                    permute_rows(1, 1, r * KC)
            return 0
        with scope("q"):
            lax.fori_loop(0, NQM, q_body, 0)

        def kv_body(it, _):
            m = 1 + it // NQM
            r = it % NQM
            @pl.when(m < 2)
            def _():
                with scope("wwv"):
                    wkv_copy(2, r).wait()
            r0 = pl.multiple_of(r * QM, QM)
            wmat = pltpu.bitcast(wp_v[m], jnp.bfloat16)
            xn = pltpu.bitcast(xn_v[pl.ds(pl.multiple_of(r0 // 2, QM // 2), QM // 2), :], jnp.bfloat16)
            res = jnp.dot(xn, wmat, preferred_element_type=jnp.float32)
            for t in range(NT):
                kv_s[(m - 1) * NT + t, pl.ds(r0 + HALO, QM), :] = res[:, t * 128:(t + 1) * 128]
            permute_rows(2, m + 1, r * KC)
            for p0 in range(0, QP, QPR):
                rws = pl.ds(pl.multiple_of(it * QP + p0, QPR), QPR)
                mu = st_s[0, rws, :]
                rs = st_s[1, rws, :]
                us = []
                for t in range(NT):
                    cst = jnp.broadcast_to(cs_s[0:1, t * 128:(t + 1) * 128], (QPR, 128))
                    qn = (q_s[t, rws, :] - mu * cst) * rs
                    us.append(pltpu.bitcast(qn.astype(jnp.bfloat16), jnp.uint32))
                ys = _swap_heads(us)
                for t in range(NT):
                    q_s[t, rws, :] = pltpu.bitcast(ys[t], jnp.bfloat16).astype(jnp.float32)
            return 0
        with scope("kv"):
            lax.fori_loop(0, 2 * NQM, kv_body, 0)

        with scope("wwait"):
            for cp in w_copies:
                cp.wait()

        def main_body(i, _):
            base = pl.multiple_of(i * BM, BM)
            rows = pl.ds(base, BM)

            def attn_rows(r0):
                b0 = base + (HALO + r0)
                q = [q_s[t, pl.ds(base + r0, RB), :] for t in range(NT)]
                lg = []
                for w in range(W):
                    p = None
                    for t in range(NT):
                        pr = q[t] * kv_s[t, pl.ds(b0 - DIL * w, RB), :]
                        p = pr if p is None else p + pr
                    p = p + pltpu.roll(p, 64, 1)
                    p = p + pltpu.roll(p, 32, 1)
                    if w > 0 and r0 < HALO:
                        row_top = lax.broadcasted_iota(jnp.int32, (HALO, 128), 0) + base
                        top = jnp.where(row_top >= DIL * w, p[:HALO], -1e9)
                        p = jnp.concatenate([top, p[HALO:]], axis=0) if RB > HALO else top
                    lg.append(p)
                mx = functools.reduce(jnp.maximum, lg)
                e = [jnp.exp2(l - mx) for l in lg]
                den = functools.reduce(lambda a, b: a + b, e)
                rinv = pltpu.reciprocal(den, approx=True)
                e = [ew * rinv for ew in e]
                os_ = []
                for t in range(NT):
                    o = None
                    for w in range(W):
                        ov = e[w] * kv_s[NT + t, pl.ds(b0 - DIL * w, RB), :]
                        o = ov if o is None else o + ov
                    os_.append(pltpu.bitcast(o.astype(jnp.bfloat16), jnp.uint32))
                return jnp.concatenate(_swap_heads(os_), axis=1)

            xu = xn_v[pl.ds(pl.multiple_of(base // 2, BM // 2), BM // 2), :]
            xn = pltpu.bitcast(xu, jnp.bfloat16)
            pieces = list(range(0, BM, RB))
            keep = flag_s[0] > 0
            outs = [attn_rows(p) for p in pieces]
            at = {}
            for n in range(len(pieces)):
                at.setdefault(apos + n * (npin - apos) // len(pieces), []).append(n)

            def pinned(pos):
                if pos not in at:
                    return xn
                head = xu[0:8, 0:128]
                for n in at[pos]:
                    head = jnp.where(keep, head, outs[n][0:8, 0:128])
                top = jnp.concatenate([head, xu[0:8, 128:]], axis=1)
                return pltpu.bitcast(jnp.concatenate([top, xu[8:]], axis=0), jnp.bfloat16)

            acc = None
            for c in range(NF):
                cs = slice(c * BF, (c + 1) * BF)
                g = jnp.dot(pinned(2 * c), wg_v[:, cs], preferred_element_type=jnp.float32)
                u = jnp.dot(pinned(2 * c + 1), wu_v[:, cs], preferred_element_type=jnp.float32)
                h = (g * _sigmoid(g) * u).astype(jnp.bfloat16)
                d = jnp.dot(h, wd_v[cs, :], preferred_element_type=jnp.float32)
                acc = d if acc is None else acc + d
            o = pltpu.bitcast(jnp.concatenate(outs, axis=0), jnp.bfloat16)
            s = jnp.dot(o, wo_v[...], preferred_element_type=jnp.float32)
            gy = acc * _sigmoid(acc)
            out_v[rows, :] = (in_v[rows, :].astype(jnp.float32) + s * gy).astype(out_v.dtype)
            out_copy(i).start()
            return 0
        with scope("main"):
            lax.fori_loop(0, NSTEP, main_body, 0)
        for i in range(NSTEP):
            out_copy(i).wait()

    def fn(A_x, A_wqkv, A_wo, B_x, B_w_gate, B_w_up, B_w_down):
        x = A_x.reshape(S, D)
        any_spec = pl.BlockSpec(memory_space=pl.ANY)
        out = pl.pallas_call(
            kernel,
            in_specs=[any_spec] * 6,
            out_specs=any_spec,
            out_shape=jax.ShapeDtypeStruct((S, D), jnp.bfloat16),
            scratch_shapes=[
                pltpu.VMEM((S + 3 * D, D), jnp.bfloat16),
                pltpu.VMEM((S // 2, D), jnp.uint32),
                pltpu.VMEM((4, D // 2, D), jnp.uint32),
                pltpu.VMEM((D, D), jnp.bfloat16),
                pltpu.VMEM((D, F), jnp.bfloat16),
                pltpu.VMEM((D, F), jnp.bfloat16),
                pltpu.VMEM((F, D), jnp.bfloat16),
                pltpu.VMEM((2 * NT, HALO + S, 128), jnp.float32),
                pltpu.VMEM((NT, S, 128), jnp.float32),
                pltpu.VMEM((2, S, 128), jnp.float32),
                pltpu.VMEM((8, D), jnp.float32),
                pltpu.VMEM((S, D), jnp.bfloat16),
                pltpu.SMEM((1,), jnp.int32),
                pltpu.SemaphoreType.DMA((NQM,)),
                pltpu.SemaphoreType.DMA((len(first),)),
                pltpu.SemaphoreType.DMA((2 * NQM,)),
                pltpu.SemaphoreType.DMA((4,)),
                pltpu.SemaphoreType.DMA((NSTEP,)),
            ],
            compiler_params=pltpu.CompilerParams(vmem_limit_bytes=120 * 1024 * 1024,
                                                 disable_semaphore_checks=nosem, disable_bounds_checks=nobounds),
        )(x, A_wqkv, A_wo, B_w_gate, B_w_up, B_w_down)
        return out.reshape(1, S, D)
    return fn


@jax.jit
def pallas_recurrent_scan__sliding_local_dilated__swiglu_ffn__prompt_kernel(
    A_x: jax.Array,
    A_wqkv: jax.Array,
    A_wo: jax.Array,
    B_x: jax.Array,
    B_w_gate: jax.Array,
    B_w_up: jax.Array,
    B_w_down: jax.Array,
):
    return make(nosem=True)(A_x, A_wqkv, A_wo, B_x, B_w_gate, B_w_up, B_w_down)
```

```python
import functools

import jax
import jax.numpy as jnp
import jax.experimental.pallas as pl
import jax.experimental.pallas.tpu as pltpu
from jax import lax

S, D, F = 2048, 1024, 3584
DH, W, DIL = 32, 8, 2
HALO = 16
NT = D // 128
LOG2E = 1.4426950408889634
QSCALE = DH ** -0.5 * LOG2E

BM = 256
BF = 512
RB = 16
QM = 512
QSEG = (384, 640)
QROWS, QCOLS = 128, 128
LNR = 16
QPR = 64
PR = 128
OSPLIT = 8

NSTEP = S // BM
NF = F // BF
NQM = S // QM
KC = D // NQM
WQ0 = S


def _sigmoid(x):
    return pltpu.reciprocal(1.0 + jnp.exp2(x * (-LOG2E)), approx=True)


def _swap_heads(xs):
    lane = lax.broadcasted_iota(jnp.int32, xs[0].shape, 1)
    g = lane >> 4
    e = lane & 15
    zs = []
    for s in range(NT):
        idx = (e & 3) * 32 + ((g - s) & 7) * 4 + (e >> 2)
        zs.append(jnp.take_along_axis(xs[s], idx, axis=1, mode="promise_in_bounds"))
    a = [zs[(-t) % NT] for t in range(NT)]
    for b in range(3):
        bit = ((g >> b) & 1) == 1
        a = [jnp.where(bit, a[(t - (1 << b)) % NT], a[t]) for t in range(NT)]
    out = []
    for t in range(NT):
        idx = ((((lane >> 2) & 7) + t) & 7) * 16 + (lane >> 5) * 4 + (lane & 3)
        out.append(jnp.take_along_axis(a[t], idx, axis=1, mode="promise_in_bounds"))
    return out


def _bf16_words(x):
    return pltpu.bitcast(x.astype(jnp.bfloat16), jnp.uint32)


def _kernel(x_h, wqkv_h, wo_h, wg_h, wu_h, wd_h, out_h,
            in_v, xn_v, wp_v, wo_v, wg_v, wu_v, wd_v, kv_s, q_s, st_s, cs_s, out_v,
            sem_x, sem_q, sem_kv, sem_w, sem_out):
    def x_copy(r):
        return pltpu.make_async_copy(x_h.at[pl.ds(r * QM, QM), :], in_v.at[pl.ds(r * QM, QM), :], sem_x.at[r])

    def wq_copy(i):
        c0 = sum(QSEG[:i])
        return pltpu.make_async_copy(wqkv_h.at[:, pl.ds(c0, QSEG[i])],
                                     in_v.at[pl.ds(WQ0, D), pl.ds(c0, QSEG[i])], sem_q.at[i])

    def wkv_copy(m, r):
        return pltpu.make_async_copy(wqkv_h.at[pl.ds(r * KC, KC), pl.ds(m * D, D)],
                                     in_v.at[pl.ds(WQ0 + m * D + r * KC, KC), :], sem_kv.at[(m - 1) * NQM + r])

    w_copies = [pltpu.make_async_copy(src, dst, sem_w.at[n])
                for n, (src, dst) in enumerate([(wg_h, wg_v), (wu_h, wu_v), (wd_h, wd_v), (wo_h, wo_v)])]

    def out_copy(i, j):
        cw = D // OSPLIT
        return pltpu.make_async_copy(out_v.at[pl.ds(i * BM, BM), pl.ds(j * cw, cw)],
                                     out_h.at[pl.ds(i * BM, BM), pl.ds(j * cw, cw)], sem_out.at[i * OSPLIT + j])

    def permute_weight_rows(ms, md, k0):
        for p0 in range(0, KC, 2 * PR):
            src = in_v[pl.ds(pl.multiple_of(WQ0 + ms * D + k0 + p0, 2 * PR), 2 * PR), :]
            u = pltpu.bitcast(src, jnp.uint32)
            ys = _swap_heads([u[:, s * 128:(s + 1) * 128] for s in range(NT)])
            dst0 = pl.multiple_of((k0 + p0) // 2, PR)
            for t in range(NT):
                wp_v[md, pl.ds(dst0, PR), t * 128:(t + 1) * 128] = ys[t]

    x_copy(0).start()
    for i in range(len(QSEG)):
        wq_copy(i).start()
    wkv_copy(1, 0).start()
    for r in range(1, NQM):
        x_copy(r).start()
        wkv_copy(1, r).start()
    for r in range(NQM):
        wkv_copy(2, r).start()
    kv_s[:, 0:HALO, :] = jnp.zeros((2 * NT, HALO, 128), jnp.float32)

    def layernorm_piece(r0):
        rows = pl.ds(pl.multiple_of(r0, LNR), LNR)
        x = in_v[rows, :].astype(jnp.float32)
        mu = jnp.mean(x, axis=-1, keepdims=True)
        xc = x - mu
        var = jnp.mean(xc * xc, axis=-1, keepdims=True)
        rs = lax.rsqrt(var + 1e-5)
        xn = _bf16_words(xc * rs)
        xn_v[pl.ds(pl.multiple_of(r0 // 2, LNR // 2), LNR // 2), :] = xn
        st_s[0, rows, :] = jnp.broadcast_to(mu, (LNR, 128))
        st_s[1, rows, :] = jnp.broadcast_to(rs * QSCALE, (LNR, 128))
        return xn

    def q_body(r, carry):
        r0 = pl.multiple_of(r * QM, QM)
        npc = QM // LNR
        for i, cw in enumerate(QSEG):
            last = i == len(QSEG) - 1
            c0 = sum(QSEG[:i])
            if i == 0:
                x_copy(r).wait()
            if last:
                wkv_copy(1, r).wait()

            @pl.when(r == 0)
            def _():
                wq_copy(i).wait()

            if last:
                @pl.when(r == 1)
                def _():
                    for cp in w_copies:
                        cp.start()

            keep = (pltpu.bitcast(in_v[pl.ds(r0, 16), 0:128], jnp.uint32) | 1) != 0
            subs = [(j, h) for j in range(cw // QCOLS) for h in range(QM // QROWS)]
            xbs = [in_v[pl.ds(pl.multiple_of(r0 + h * QROWS, QROWS), QROWS), :] for h in range(QM // QROWS)]
            mine = [n for n in range(npc) if c0 <= n * D // npc < c0 + cw]
            xns = {n: layernorm_piece(r0 + n * LNR) for n in mine}
            for k, (j, h) in enumerate(subs):
                lhs = xb = xbs[h]
                tied = [n for kk, n in enumerate(mine) if 1 + kk * len(subs) // len(mine) == k]
                if tied:
                    head = pltpu.bitcast(xb[0:16, 0:128], jnp.uint32)
                    for n in tied:
                        head = jnp.where(keep, head, xns[n][0:8, 0:128])
                    top = jnp.concatenate([pltpu.bitcast(head, jnp.bfloat16), xb[0:16, 128:]], axis=1)
                    lhs = jnp.concatenate([top, xb[16:]], axis=0)
                cols = slice(c0 + j * QCOLS, c0 + (j + 1) * QCOLS)
                res = jnp.dot(lhs, in_v[WQ0:WQ0 + D, cols], preferred_element_type=jnp.float32)
                q_s[cols.start // 128, pl.ds(pl.multiple_of(r0 + h * QROWS, QROWS), QROWS), :] = res
            if last:
                ccols = pl.ds(pl.multiple_of(r * (D // NQM), D // NQM), D // NQM)
                cs = jnp.sum(in_v[WQ0:WQ0 + D, ccols].astype(jnp.float32), axis=0, keepdims=True)
                cs_s[:, ccols] = jnp.broadcast_to(cs, (8, D // NQM))
                permute_weight_rows(1, 1, r * KC)
        return carry

    lax.fori_loop(0, NQM, q_body, 0)

    QP = S // (2 * NQM)

    def kv_body(it, carry):
        m = 1 + it // NQM
        r = it % NQM

        @pl.when(m < 2)
        def _():
            wkv_copy(2, r).wait()

        r0 = pl.multiple_of(r * QM, QM)
        wmat = pltpu.bitcast(wp_v[m], jnp.bfloat16)
        xn = pltpu.bitcast(xn_v[pl.ds(pl.multiple_of(r0 // 2, QM // 2), QM // 2), :], jnp.bfloat16)
        res = jnp.dot(xn, wmat, preferred_element_type=jnp.float32)
        for t in range(NT):
            kv_s[(m - 1) * NT + t, pl.ds(r0 + HALO, QM), :] = res[:, t * 128:(t + 1) * 128]
        permute_weight_rows(2, m + 1, r * KC)
        for p0 in range(0, QP, QPR):
            rows = pl.ds(pl.multiple_of(it * QP + p0, QPR), QPR)
            mu = st_s[0, rows, :]
            rs = st_s[1, rows, :]
            us = []
            for t in range(NT):
                cst = jnp.broadcast_to(cs_s[0:1, t * 128:(t + 1) * 128], (QPR, 128))
                us.append(_bf16_words((q_s[t, rows, :] - mu * cst) * rs))
            ys = _swap_heads(us)
            for t in range(NT):
                q_s[t, rows, :] = pltpu.bitcast(ys[t], jnp.bfloat16).astype(jnp.float32)
        return carry

    lax.fori_loop(0, 2 * NQM, kv_body, 0)

    for cp in w_copies:
        cp.wait()

    def main_body(i, carry):
        base = pl.multiple_of(i * BM, BM)
        rows = pl.ds(base, BM)

        def attention_piece(r0):
            b0 = base + (HALO + r0)
            q = [q_s[t, pl.ds(base + r0, RB), :] for t in range(NT)]
            lg = []
            for w in range(W):
                p = None
                for t in range(NT):
                    pr = q[t] * kv_s[t, pl.ds(b0 - DIL * w, RB), :]
                    p = pr if p is None else p + pr
                p = p + pltpu.roll(p, 64, 1)
                p = p + pltpu.roll(p, 32, 1)
                if w > 0 and r0 < HALO:
                    pos = lax.broadcasted_iota(jnp.int32, (RB, 128), 0) + (base + r0)
                    p = jnp.where(pos >= DIL * w, p, -1e9)
                lg.append(p)
            mx = functools.reduce(jnp.maximum, lg)
            e = [jnp.exp2(l - mx) for l in lg]
            den = functools.reduce(lambda a, b: a + b, e)
            rinv = pltpu.reciprocal(den, approx=True)
            e = [ew * rinv for ew in e]
            os_ = []
            for t in range(NT):
                o = None
                for w in range(W):
                    ov = e[w] * kv_s[NT + t, pl.ds(b0 - DIL * w, RB), :]
                    o = ov if o is None else o + ov
                os_.append(_bf16_words(o))
            return jnp.concatenate(_swap_heads(os_), axis=1)

        xu = xn_v[pl.ds(pl.multiple_of(base // 2, BM // 2), BM // 2), :]
        xn = pltpu.bitcast(xu, jnp.bfloat16)
        outs = [attention_piece(r0) for r0 in range(0, BM, RB)]
        keep = (xu[0:8, 0:128] | 1) != 0

        def lhs_for(pos):
            tied = [n for n in range(len(outs)) if 1 + n * (2 * NF - 1) // len(outs) == pos]
            if not tied:
                return xn
            head = xu[0:8, 0:128]
            for n in tied:
                head = jnp.where(keep, head, outs[n][0:8, 0:128])
            top = jnp.concatenate([head, xu[0:8, 128:]], axis=1)
            return pltpu.bitcast(jnp.concatenate([top, xu[8:]], axis=0), jnp.bfloat16)

        acc = None
        for c in range(NF):
            cs = slice(c * BF, (c + 1) * BF)
            g = jnp.dot(lhs_for(2 * c), wg_v[:, cs], preferred_element_type=jnp.float32)
            u = jnp.dot(lhs_for(2 * c + 1), wu_v[:, cs], preferred_element_type=jnp.float32)
            h = (g * _sigmoid(g) * u).astype(jnp.bfloat16)
            d = jnp.dot(h, wd_v[cs, :], preferred_element_type=jnp.float32)
            acc = d if acc is None else acc + d
        o = pltpu.bitcast(jnp.concatenate(outs, axis=0), jnp.bfloat16)
        s = jnp.dot(o, wo_v[...], preferred_element_type=jnp.float32)
        gy = acc * _sigmoid(acc)
        cw = D // OSPLIT
        for j in range(OSPLIT):
            cols = slice(j * cw, (j + 1) * cw)
            out_v[rows, cols] = (in_v[rows, cols].astype(jnp.float32) + s[:, cols] * gy[:, cols]).astype(out_v.dtype)
            out_copy(i, j).start()
        return carry

    lax.fori_loop(0, NSTEP, main_body, 0)
    for i in range(NSTEP):
        for j in range(OSPLIT):
            out_copy(i, j).wait()


def _run(A_x, A_wqkv, A_wo, B_x, B_w_gate, B_w_up, B_w_down):
    del B_x
    hbm = pl.BlockSpec(memory_space=pl.ANY)
    out = pl.pallas_call(
        _kernel,
        in_specs=[hbm] * 6,
        out_specs=hbm,
        out_shape=jax.ShapeDtypeStruct((S, D), jnp.bfloat16),
        scratch_shapes=[
            pltpu.VMEM((S + 3 * D, D), jnp.bfloat16),
            pltpu.VMEM((S // 2, D), jnp.uint32),
            pltpu.VMEM((4, D // 2, D), jnp.uint32),
            pltpu.VMEM((D, D), jnp.bfloat16),
            pltpu.VMEM((D, F), jnp.bfloat16),
            pltpu.VMEM((D, F), jnp.bfloat16),
            pltpu.VMEM((F, D), jnp.bfloat16),
            pltpu.VMEM((2 * NT, HALO + S, 128), jnp.float32),
            pltpu.VMEM((NT, S, 128), jnp.float32),
            pltpu.VMEM((2, S, 128), jnp.float32),
            pltpu.VMEM((8, D), jnp.float32),
            pltpu.VMEM((S, D), jnp.bfloat16),
            pltpu.SemaphoreType.DMA((NQM,)),
            pltpu.SemaphoreType.DMA((len(QSEG),)),
            pltpu.SemaphoreType.DMA((2 * NQM,)),
            pltpu.SemaphoreType.DMA((4,)),
            pltpu.SemaphoreType.DMA((NSTEP * OSPLIT,)),
        ],
        compiler_params=pltpu.CompilerParams(vmem_limit_bytes=120 * 1024 * 1024, disable_semaphore_checks=True),
    )(A_x.reshape(S, D), A_wqkv, A_wo, B_w_gate, B_w_up, B_w_down)
    return out.reshape(1, S, D)


@jax.jit
def pallas_recurrent_scan__sliding_local_dilated__swiglu_ffn__prompt_kernel(
    A_x: jax.Array,
    A_wqkv: jax.Array,
    A_wo: jax.Array,
    B_x: jax.Array,
    B_w_gate: jax.Array,
    B_w_up: jax.Array,
    B_w_down: jax.Array,
):
    return _run(A_x, A_wqkv, A_wo, B_x, B_w_gate, B_w_up, B_w_down)
```

```python
import functools

import numpy as np
import jax
import jax.numpy as jnp
import jax.experimental.pallas as pl
import jax.experimental.pallas.tpu as pltpu
from jax import lax

S, D, F = 2048, 1024, 3584
DH, W, DIL = 32, 8, 2
HALO = 16
NT = D // 128
LOG2E = 1.4426950408889634
QSCALE = DH ** -0.5 * LOG2E

BM = 256
BF = 512
RB = 16
QM = 512
QSEG = (384, 640)
QROWS, QCOLS = 128, 128
LNR = 16
QPR = 64
PR = 128
WOPIN, WOSTEP = 0, 2
OSPLIT = 8

NSTEP = S // BM
NF = F // BF
NQM = S // QM
KC = D // NQM
WQ0 = S
WO0 = S + 3 * D


def _sigmoid(x):
    return pltpu.reciprocal(1.0 + jnp.exp2(x * (-LOG2E)), approx=True)


def _swap_heads(xs):
    lane = lax.broadcasted_iota(jnp.int32, xs[0].shape, 1)
    g = lane >> 4
    e = lane & 15
    zs = []
    for s in range(NT):
        idx = (e & 3) * 32 + ((g - s) & 7) * 4 + (e >> 2)
        zs.append(jnp.take_along_axis(xs[s], idx, axis=1, mode="promise_in_bounds"))
    a = [zs[(-t) % NT] for t in range(NT)]
    for b in range(3):
        bit = ((g >> b) & 1) == 1
        a = [jnp.where(bit, a[(t - (1 << b)) % NT], a[t]) for t in range(NT)]
    out = []
    for t in range(NT):
        idx = ((((lane >> 2) & 7) + t) & 7) * 16 + (lane >> 5) * 4 + (lane & 3)
        out.append(jnp.take_along_axis(a[t], idx, axis=1, mode="promise_in_bounds"))
    return out


def _transpose_sublanes(xs):
    p = lax.broadcasted_iota(jnp.int32, xs[0].shape, 0)
    ys = [x if i == 0 else pltpu.roll(x, i, 0) for i, x in enumerate(xs)]
    a = [ys[(-t) % 8] for t in range(8)]
    for b in range(3):
        bit = ((p >> b) & 1) == 1
        a = [jnp.where(bit, a[(t - (1 << b)) % 8], a[t]) for t in range(8)]
    return [x if s == 0 else pltpu.roll(x, 8 - s, 0) for s, x in enumerate(a)]


def _bf16_words(x):
    return pltpu.bitcast(x.astype(jnp.bfloat16), jnp.uint32)


def _kernel(x_h, wqkv_h, wo_h, wg_h, wu_h, wd_h, out_h,
            in_v, xn_v, wp_v, wop_v, wg_v, wu_v, wd_v, kv_s, q_s, st_s, cs_s, out_v,
            sem_x, sem_q, sem_kv, sem_w, sem_out):
    def x_copy(r):
        return pltpu.make_async_copy(x_h.at[pl.ds(r * QM, QM), :], in_v.at[pl.ds(r * QM, QM), :], sem_x.at[r])

    def wq_copy(i):
        c0 = sum(QSEG[:i])
        return pltpu.make_async_copy(wqkv_h.at[:, pl.ds(c0, QSEG[i])],
                                     in_v.at[pl.ds(WQ0, D), pl.ds(c0, QSEG[i])], sem_q.at[i])

    def wkv_copy(m, r):
        return pltpu.make_async_copy(wqkv_h.at[pl.ds(r * KC, KC), pl.ds(m * D, D)],
                                     in_v.at[pl.ds(WQ0 + m * D + r * KC, KC), :], sem_kv.at[(m - 1) * NQM + r])

    w_copies = [pltpu.make_async_copy(src, dst, sem_w.at[n])
                for n, (src, dst) in enumerate([(wg_h, wg_v), (wu_h, wu_v), (wd_h, wd_v)])]
    wo_copy = pltpu.make_async_copy(wo_h, in_v.at[pl.ds(WO0, D), :], sem_w.at[3])

    def out_copy(i, j):
        cw = D // OSPLIT
        return pltpu.make_async_copy(out_v.at[pl.ds(i * BM, BM), pl.ds(j * cw, cw)],
                                     out_h.at[pl.ds(i * BM, BM), pl.ds(j * cw, cw)], sem_out.at[i * OSPLIT + j])

    def permute_weight_rows(ms, md, k0):
        for p0 in range(0, KC, 2 * PR):
            src = in_v[pl.ds(pl.multiple_of(WQ0 + ms * D + k0 + p0, 2 * PR), 2 * PR), :]
            u = pltpu.bitcast(src, jnp.uint32)
            ys = _swap_heads([u[:, s * 128:(s + 1) * 128] for s in range(NT)])
            dst0 = pl.multiple_of((k0 + p0) // 2, PR)
            for t in range(NT):
                wp_v[md, pl.ds(dst0, PR), t * 128:(t + 1) * 128] = ys[t]

    x_copy(0).start()
    for i in range(len(QSEG)):
        wq_copy(i).start()
    wkv_copy(1, 0).start()
    for r in range(1, NQM):
        x_copy(r).start()
        wkv_copy(1, r).start()
    for r in range(NQM):
        wkv_copy(2, r).start()
    wo_copy.start()
    kv_s[:, 0:HALO, :] = jnp.zeros((2 * NT, HALO, 128), jnp.float32)

    def layernorm_piece(r0):
        rows = pl.ds(pl.multiple_of(r0, LNR), LNR)
        x = in_v[rows, :].astype(jnp.float32)
        mu = jnp.mean(x, axis=-1, keepdims=True)
        xc = x - mu
        var = jnp.mean(xc * xc, axis=-1, keepdims=True)
        rs = lax.rsqrt(var + 1e-5)
        xn = _bf16_words(xc * rs)
        xn_v[pl.ds(pl.multiple_of(r0 // 2, LNR // 2), LNR // 2), :] = xn
        st_s[0, rows, :] = jnp.broadcast_to(mu, (LNR, 128))
        st_s[1, rows, :] = jnp.broadcast_to(rs * QSCALE, (LNR, 128))
        return xn

    def q_body(r, carry):
        r0 = pl.multiple_of(r * QM, QM)
        npc = QM // LNR
        for i, cw in enumerate(QSEG):
            last = i == len(QSEG) - 1
            c0 = sum(QSEG[:i])
            if i == 0:
                x_copy(r).wait()
            if last:
                wkv_copy(1, r).wait()

            @pl.when(r == 0)
            def _():
                wq_copy(i).wait()

            if last:
                @pl.when(r == 1)
                def _():
                    for cp in w_copies:
                        cp.start()

            keep = (pltpu.bitcast(in_v[pl.ds(r0, 16), 0:128], jnp.uint32) | 1) != 0
            subs = [(j, h) for j in range(cw // QCOLS) for h in range(QM // QROWS)]
            xbs = [in_v[pl.ds(pl.multiple_of(r0 + h * QROWS, QROWS), QROWS), :] for h in range(QM // QROWS)]
            mine = [n for n in range(npc) if c0 <= n * D // npc < c0 + cw]
            xns = {n: layernorm_piece(r0 + n * LNR) for n in mine}
            for k, (j, h) in enumerate(subs):
                lhs = xb = xbs[h]
                tied = [n for kk, n in enumerate(mine) if 1 + kk * len(subs) // len(mine) == k]
                if tied:
                    head = pltpu.bitcast(xb[0:16, 0:128], jnp.uint32)
                    for n in tied:
                        head = jnp.where(keep, head, xns[n][0:8, 0:128])
                    top = jnp.concatenate([pltpu.bitcast(head, jnp.bfloat16), xb[0:16, 128:]], axis=1)
                    lhs = jnp.concatenate([top, xb[16:]], axis=0)
                cols = slice(c0 + j * QCOLS, c0 + (j + 1) * QCOLS)
                res = jnp.dot(lhs, in_v[WQ0:WQ0 + D, cols], preferred_element_type=jnp.float32)
                q_s[cols.start // 128, pl.ds(pl.multiple_of(r0 + h * QROWS, QROWS), QROWS), :] = res
            if last:
                ccols = pl.ds(pl.multiple_of(r * (D // NQM), D // NQM), D // NQM)
                cs = jnp.sum(in_v[WQ0:WQ0 + D, ccols].astype(jnp.float32), axis=0, keepdims=True)
                cs_s[:, ccols] = jnp.broadcast_to(cs, (8, D // NQM))
                permute_weight_rows(1, 1, r * KC)
        return carry

    lax.fori_loop(0, NQM, q_body, 0)

    QP = S // (2 * NQM)
    wo_copy.wait()

    def permute_wo_rows(t, res):
        cols = pl.ds(pl.multiple_of(t * 128, 128), 128)
        u = pltpu.bitcast(in_v[WO0:WO0 + D, cols], jnp.uint32)
        keep = (u[0:8] | 1) != 0
        for b in range(2):
            for dh in range(2):
                g = 2 * b + dh
                after = pltpu.bitcast(res[0:8, (WOPIN + WOSTEP * g) * 128:(WOPIN + WOSTEP * g + 1) * 128], jnp.uint32)
                xa = [u[8 * (4 * (8 * b + i) + dh):8 * (4 * (8 * b + i) + dh) + 8] for i in range(8)]
                xc = [u[8 * (4 * (8 * b + i) + 2 + dh):8 * (4 * (8 * b + i) + 2 + dh) + 8] for i in range(8)]
                if WOPIN >= 0:
                    xa[0] = jnp.where(keep, xa[0], after)
                    xc[0] = jnp.where(keep, xc[0], after)
                ta = _transpose_sublanes(xa)
                tc = _transpose_sublanes(xc)
                for s_ in range(8):
                    d2 = 8 * dh + s_
                    a, c = ta[s_], tc[s_]
                    wop_v[pl.ds(32 * d2 + 8 * b, 8), cols] = (a & 0xFFFF) | (c << 16)
                    wop_v[pl.ds(32 * d2 + 16 + 8 * b, 8), cols] = (a >> 16) | (c & np.uint32(0xFFFF0000))

    def kv_body(it, carry):
        m = 1 + it // NQM
        r = it % NQM

        @pl.when(m < 2)
        def _():
            wkv_copy(2, r).wait()

        r0 = pl.multiple_of(r * QM, QM)
        wmat = pltpu.bitcast(wp_v[m], jnp.bfloat16)
        xn = pltpu.bitcast(xn_v[pl.ds(pl.multiple_of(r0 // 2, QM // 2), QM // 2), :], jnp.bfloat16)
        res = jnp.dot(xn, wmat, preferred_element_type=jnp.float32)
        for t in range(NT):
            kv_s[(m - 1) * NT + t, pl.ds(r0 + HALO, QM), :] = res[:, t * 128:(t + 1) * 128]
        permute_weight_rows(2, m + 1, r * KC)
        permute_wo_rows(it, res)
        for p0 in range(0, QP, QPR):
            rows = pl.ds(pl.multiple_of(it * QP + p0, QPR), QPR)
            mu = st_s[0, rows, :]
            rs = st_s[1, rows, :]
            us = []
            for t in range(NT):
                cst = jnp.broadcast_to(cs_s[0:1, t * 128:(t + 1) * 128], (QPR, 128))
                us.append(_bf16_words((q_s[t, rows, :] - mu * cst) * rs))
            ys = _swap_heads(us)
            for t in range(NT):
                q_s[t, rows, :] = pltpu.bitcast(ys[t], jnp.bfloat16).astype(jnp.float32)
        return carry

    lax.fori_loop(0, 2 * NQM, kv_body, 0)

    for cp in w_copies:
        cp.wait()

    def main_body(i, carry):
        base = pl.multiple_of(i * BM, BM)
        rows = pl.ds(base, BM)

        def attention_piece(r0):
            b0 = base + (HALO + r0)
            q = [q_s[t, pl.ds(base + r0, RB), :] for t in range(NT)]
            lg = []
            for w in range(W):
                p = None
                for t in range(NT):
                    pr = q[t] * kv_s[t, pl.ds(b0 - DIL * w, RB), :]
                    p = pr if p is None else p + pr
                p = p + pltpu.roll(p, 64, 1)
                p = p + pltpu.roll(p, 32, 1)
                if w > 0 and r0 < HALO:
                    pos = lax.broadcasted_iota(jnp.int32, (RB, 128), 0) + (base + r0)
                    p = jnp.where(pos >= DIL * w, p, -1e9)
                lg.append(p)
            mx = functools.reduce(jnp.maximum, lg)
            e = [jnp.exp2(l - mx) for l in lg]
            den = functools.reduce(lambda a, b: a + b, e)
            rinv = pltpu.reciprocal(den, approx=True)
            e = [ew * rinv for ew in e]
            os_ = []
            for t in range(NT):
                o = None
                for w in range(W):
                    ov = e[w] * kv_s[NT + t, pl.ds(b0 - DIL * w, RB), :]
                    o = ov if o is None else o + ov
                os_.append(o)
            return jnp.concatenate(os_, axis=1).astype(jnp.bfloat16)

        xu = xn_v[pl.ds(pl.multiple_of(base // 2, BM // 2), BM // 2), :]
        xn = pltpu.bitcast(xu, jnp.bfloat16)
        outs = [attention_piece(r0) for r0 in range(0, BM, RB)]
        keep = (xu[0:8, 0:128] | 1) != 0

        def lhs_for(pos):
            tied = [n for n in range(len(outs)) if 1 + n * (2 * NF - 1) // len(outs) == pos]
            if not tied:
                return xn
            head = xu[0:8, 0:128]
            for n in tied:
                head = jnp.where(keep, head, pltpu.bitcast(outs[n][0:16, 0:128], jnp.uint32))
            top = jnp.concatenate([head, xu[0:8, 128:]], axis=1)
            return pltpu.bitcast(jnp.concatenate([top, xu[8:]], axis=0), jnp.bfloat16)

        acc = None
        for c in range(NF):
            cs = slice(c * BF, (c + 1) * BF)
            g = jnp.dot(lhs_for(2 * c), wg_v[:, cs], preferred_element_type=jnp.float32)
            u = jnp.dot(lhs_for(2 * c + 1), wu_v[:, cs], preferred_element_type=jnp.float32)
            h = (g * _sigmoid(g) * u).astype(jnp.bfloat16)
            d = jnp.dot(h, wd_v[cs, :], preferred_element_type=jnp.float32)
            acc = d if acc is None else acc + d
        o = jnp.concatenate(outs, axis=0)
        s = jnp.dot(o, pltpu.bitcast(wop_v[...], jnp.bfloat16), preferred_element_type=jnp.float32)
        gy = acc * _sigmoid(acc)
        cw = D // OSPLIT
        for j in range(OSPLIT):
            cols = slice(j * cw, (j + 1) * cw)
            out_v[rows, cols] = (in_v[rows, cols].astype(jnp.float32) + s[:, cols] * gy[:, cols]).astype(out_v.dtype)
            out_copy(i, j).start()
        return carry

    lax.fori_loop(0, NSTEP, main_body, 0)
    for i in range(NSTEP):
        for j in range(OSPLIT):
            out_copy(i, j).wait()


def _run(A_x, A_wqkv, A_wo, B_x, B_w_gate, B_w_up, B_w_down):
    del B_x
    hbm = pl.BlockSpec(memory_space=pl.ANY)
    out = pl.pallas_call(
        _kernel,
        in_specs=[hbm] * 6,
        out_specs=hbm,
        out_shape=jax.ShapeDtypeStruct((S, D), jnp.bfloat16),
        scratch_shapes=[
            pltpu.VMEM((S + 4 * D, D), jnp.bfloat16),
            pltpu.VMEM((S // 2, D), jnp.uint32),
            pltpu.VMEM((4, D // 2, D), jnp.uint32),
            pltpu.VMEM((D // 2, D), jnp.uint32),
            pltpu.VMEM((D, F), jnp.bfloat16),
            pltpu.VMEM((D, F), jnp.bfloat16),
            pltpu.VMEM((F, D), jnp.bfloat16),
            pltpu.VMEM((2 * NT, HALO + S, 128), jnp.float32),
            pltpu.VMEM((NT, S, 128), jnp.float32),
            pltpu.VMEM((2, S, 128), jnp.float32),
            pltpu.VMEM((8, D), jnp.float32),
            pltpu.VMEM((S, D), jnp.bfloat16),
            pltpu.SemaphoreType.DMA((NQM,)),
            pltpu.SemaphoreType.DMA((len(QSEG),)),
            pltpu.SemaphoreType.DMA((2 * NQM,)),
            pltpu.SemaphoreType.DMA((4,)),
            pltpu.SemaphoreType.DMA((NSTEP * OSPLIT,)),
        ],
        compiler_params=pltpu.CompilerParams(vmem_limit_bytes=120 * 1024 * 1024, disable_semaphore_checks=True),
    )(A_x.reshape(S, D), A_wqkv, A_wo, B_w_gate, B_w_up, B_w_down)
    return out.reshape(1, S, D)


@jax.jit
def pallas_recurrent_scan__sliding_local_dilated__swiglu_ffn__prompt_kernel(
    A_x: jax.Array,
    A_wqkv: jax.Array,
    A_wo: jax.Array,
    B_x: jax.Array,
    B_w_gate: jax.Array,
    B_w_up: jax.Array,
    B_w_down: jax.Array,
):
    return _run(A_x, A_wqkv, A_wo, B_x, B_w_gate, B_w_up, B_w_down)
```

```python
import functools

import numpy as np
import jax
import jax.numpy as jnp
import jax.experimental.pallas as pl
import jax.experimental.pallas.tpu as pltpu
from jax import lax

S, D, F = 2048, 1024, 3584
DH, W, DIL = 32, 8, 2
HALO = 16
NT = D // 128
LOG2E = 1.4426950408889634
QSCALE = DH ** -0.5 * LOG2E

BM = 256
BF = 512
RB = 16
QM = 512
QSEG = (384, 640)
QROWS, QCOLS = 128, 128
LNR = 16
QPR = 64
PR = 64
OSPLIT = 8

NSTEP = S // BM
NF = F // BF
NQM = S // QM
KC = D // NQM
WQ0 = S
WO0 = S + 3 * D


def _silu(x):
    return x * pltpu.reciprocal(1.0 + jnp.exp2(x * (-LOG2E)), approx=True)


def _swap_heads(xs):
    lane = lax.broadcasted_iota(jnp.int32, xs[0].shape, 1)
    g = lane >> 4
    e = lane & 15
    zs = []
    for s in range(NT):
        idx = (e & 3) * 32 + ((g - s) & 7) * 4 + (e >> 2)
        zs.append(jnp.take_along_axis(xs[s], idx, axis=1, mode="promise_in_bounds"))
    a = [zs[(-t) % NT] for t in range(NT)]
    for b in range(3):
        bit = ((g >> b) & 1) == 1
        a = [jnp.where(bit, a[(t - (1 << b)) % NT], a[t]) for t in range(NT)]
    out = []
    for t in range(NT):
        idx = ((((lane >> 2) & 7) + t) & 7) * 16 + (lane >> 5) * 4 + (lane & 3)
        out.append(jnp.take_along_axis(a[t], idx, axis=1, mode="promise_in_bounds"))
    return out


def _transpose_sublanes(xs):
    p = lax.broadcasted_iota(jnp.int32, xs[0].shape, 0)
    ys = [x if i == 0 else pltpu.roll(x, i, 0) for i, x in enumerate(xs)]
    a = [ys[(-t) % 8] for t in range(8)]
    for b in range(3):
        bit = ((p >> b) & 1) == 1
        a = [jnp.where(bit, a[(t - (1 << b)) % 8], a[t]) for t in range(8)]
    return [x if s == 0 else pltpu.roll(x, 8 - s, 0) for s, x in enumerate(a)]


def _bf16_words(x):
    return pltpu.bitcast(x.astype(jnp.bfloat16), jnp.uint32)


def _kernel(x_h, wqkv_h, wo_h, wg_h, wu_h, wd_h, out_h,
            in_v, xn_v, wp_v, wop_v, wg_v, wu_v, wd_v, kv_s, q_s, st_s, cs_s, out_v,
            sem_x, sem_q, sem_kv, sem_w, sem_out):
    def x_copy(r):
        return pltpu.make_async_copy(x_h.at[pl.ds(r * QM, QM), :], in_v.at[pl.ds(r * QM, QM), :], sem_x.at[r])

    def wq_copy(i):
        c0 = sum(QSEG[:i])
        return pltpu.make_async_copy(wqkv_h.at[:, pl.ds(c0, QSEG[i])],
                                     in_v.at[pl.ds(WQ0, D), pl.ds(c0, QSEG[i])], sem_q.at[i])

    def wkv_copy(m, r):
        return pltpu.make_async_copy(wqkv_h.at[pl.ds(r * KC, KC), pl.ds(m * D, D)],
                                     in_v.at[pl.ds(WQ0 + m * D + r * KC, KC), :], sem_kv.at[(m - 1) * NQM + r])

    w_copies = [pltpu.make_async_copy(src, dst, sem_w.at[n])
                for n, (src, dst) in enumerate([(wg_h, wg_v), (wu_h, wu_v), (wd_h, wd_v)])]
    wo_copy = pltpu.make_async_copy(wo_h, in_v.at[pl.ds(WO0, D), :], sem_w.at[3])

    def out_copy(i, j):
        cw = D // OSPLIT
        return pltpu.make_async_copy(out_v.at[pl.ds(i * BM, BM), pl.ds(j * cw, cw)],
                                     out_h.at[pl.ds(i * BM, BM), pl.ds(j * cw, cw)], sem_out.at[0])

    def permute_weight_rows(ms, md, k0):
        for p0 in range(0, KC, 2 * PR):
            src = in_v[pl.ds(pl.multiple_of(WQ0 + ms * D + k0 + p0, 2 * PR), 2 * PR), :]
            u = pltpu.bitcast(src, jnp.uint32)
            ys = _swap_heads([u[:, s * 128:(s + 1) * 128] for s in range(NT)])
            dst0 = pl.multiple_of((k0 + p0) // 2, PR)
            for t in range(NT):
                wp_v[md, pl.ds(dst0, PR), t * 128:(t + 1) * 128] = ys[t]

    x_copy(0).start()
    for i in range(len(QSEG)):
        wq_copy(i).start()
    wkv_copy(1, 0).start()
    for r in range(1, NQM):
        x_copy(r).start()
        wkv_copy(1, r).start()
    for r in range(NQM):
        wkv_copy(2, r).start()
    wo_copy.start()
    kv_s[:, 0:HALO, :] = jnp.zeros((2 * NT, HALO, 128), jnp.float32)

    def layernorm_piece(r0):
        rows = pl.ds(pl.multiple_of(r0, LNR), LNR)
        x = in_v[rows, :].astype(jnp.float32)
        mu = jnp.mean(x, axis=-1, keepdims=True)
        xc = x - mu
        var = jnp.mean(xc * xc, axis=-1, keepdims=True)
        rs = lax.rsqrt(var + 1e-5)
        xn = _bf16_words(xc * rs)
        xn_v[pl.ds(pl.multiple_of(r0 // 2, LNR // 2), LNR // 2), :] = xn
        st_s[0, rows, :] = jnp.broadcast_to(mu, (LNR, 128))
        st_s[1, rows, :] = jnp.broadcast_to(rs * QSCALE, (LNR, 128))
        return xn

    def q_body(r, carry):
        r0 = pl.multiple_of(r * QM, QM)
        npc = QM // LNR
        for i, cw in enumerate(QSEG):
            last = i == len(QSEG) - 1
            c0 = sum(QSEG[:i])
            if i == 0:
                x_copy(r).wait()
            if last:
                wkv_copy(1, r).wait()

            @pl.when(r == 0)
            def _():
                wq_copy(i).wait()

            if last:
                @pl.when(r == 1)
                def _():
                    for cp in w_copies:
                        cp.start()

            keep = (pltpu.bitcast(in_v[pl.ds(r0, 16), 0:128], jnp.uint32) | 1) != 0
            subs = [(j, h) for j in range(cw // QCOLS) for h in range(QM // QROWS)]
            xbs = [in_v[pl.ds(pl.multiple_of(r0 + h * QROWS, QROWS), QROWS), :] for h in range(QM // QROWS)]
            mine = [n for n in range(npc) if c0 <= n * D // npc < c0 + cw]
            xns = {n: layernorm_piece(r0 + n * LNR) for n in mine}
            for k, (j, h) in enumerate(subs):
                lhs = xb = xbs[h]
                tied = [n for kk, n in enumerate(mine) if 2 + kk * (len(subs) + 2) // len(mine) == k]
                if tied:
                    head = pltpu.bitcast(xb[0:16, 0:128], jnp.uint32)
                    for n in tied:
                        head = jnp.where(keep, head, xns[n][0:8, 0:128])
                    top = jnp.concatenate([pltpu.bitcast(head, jnp.bfloat16), xb[0:16, 128:]], axis=1)
                    lhs = jnp.concatenate([top, xb[16:]], axis=0)
                cols = slice(c0 + j * QCOLS, c0 + (j + 1) * QCOLS)
                res = jnp.dot(lhs, in_v[WQ0:WQ0 + D, cols], preferred_element_type=jnp.float32)
                q_s[cols.start // 128, pl.ds(pl.multiple_of(r0 + h * QROWS, QROWS), QROWS), :] = res
            if last:
                ccols = pl.ds(pl.multiple_of(r * (D // NQM), D // NQM), D // NQM)
                cs = jnp.sum(in_v[WQ0:WQ0 + D, ccols].astype(jnp.float32), axis=0, keepdims=True)
                cs_s[:, ccols] = jnp.broadcast_to(cs, (8, D // NQM))
                permute_weight_rows(1, 1, r * KC)
        return carry

    lax.fori_loop(0, NQM, q_body, 0)

    QP = S // (2 * NQM)
    wo_copy.wait()

    def permute_wo_rows(t, res):
        cols = pl.ds(pl.multiple_of(t * 128, 128), 128)
        u = pltpu.bitcast(in_v[WO0:WO0 + D, cols], jnp.uint32)
        keep = (u[0:8] | 1) != 0
        for b in range(2):
            for dh in range(2):
                g = 2 * b + dh
                after = pltpu.bitcast(res[0:8, 2 * g * 128:(2 * g + 1) * 128], jnp.uint32)
                xa = [u[8 * (4 * (8 * b + i) + dh):8 * (4 * (8 * b + i) + dh) + 8] for i in range(8)]
                xc = [u[8 * (4 * (8 * b + i) + 2 + dh):8 * (4 * (8 * b + i) + 2 + dh) + 8] for i in range(8)]
                xa[0] = jnp.where(keep, xa[0], after)
                xc[0] = jnp.where(keep, xc[0], after)
                ta = _transpose_sublanes(xa)
                tc = _transpose_sublanes(xc)
                for s_ in range(8):
                    d2 = 8 * dh + s_
                    a, c = ta[s_], tc[s_]
                    wop_v[pl.ds(32 * d2 + 8 * b, 8), cols] = (a & 0xFFFF) | (c << 16)
                    wop_v[pl.ds(32 * d2 + 16 + 8 * b, 8), cols] = (a >> 16) | (c & np.uint32(0xFFFF0000))

    def kv_body(it, carry):
        m = 1 + it // NQM
        r = it % NQM

        @pl.when(m < 2)
        def _():
            wkv_copy(2, r).wait()

        r0 = pl.multiple_of(r * QM, QM)
        wmat = pltpu.bitcast(wp_v[m], jnp.bfloat16)
        xn = pltpu.bitcast(xn_v[pl.ds(pl.multiple_of(r0 // 2, QM // 2), QM // 2), :], jnp.bfloat16)
        res = jnp.dot(xn, wmat, preferred_element_type=jnp.float32)
        for t in range(NT):
            kv_s[(m - 1) * NT + t, pl.ds(r0 + HALO, QM), :] = res[:, t * 128:(t + 1) * 128]
        permute_weight_rows(2, m + 1, r * KC)
        permute_wo_rows(it, res)
        for p0 in range(0, QP, QPR):
            rows = pl.ds(pl.multiple_of(it * QP + p0, QPR), QPR)
            mu = st_s[0, rows, :]
            rs = st_s[1, rows, :]
            us = []
            for t in range(NT):
                cst = jnp.broadcast_to(cs_s[0:1, t * 128:(t + 1) * 128], (QPR, 128))
                us.append(_bf16_words((q_s[t, rows, :] - mu * cst) * rs))
            ys = _swap_heads(us)
            for t in range(NT):
                q_s[t, rows, :] = pltpu.bitcast(ys[t], jnp.bfloat16).astype(jnp.float32)
        return carry

    lax.fori_loop(0, 2 * NQM, kv_body, 0)

    for cp in w_copies:
        cp.wait()

    def main_body(i, carry):
        base = pl.multiple_of(i * BM, BM)
        rows = pl.ds(base, BM)

        def attention_piece(r0):
            b0 = base + (HALO + r0)
            q = [q_s[t, pl.ds(base + r0, RB), :] for t in range(NT)]
            lg = []
            for w in range(W):
                p = None
                for t in range(NT):
                    pr = q[t] * kv_s[t, pl.ds(b0 - DIL * w, RB), :]
                    p = pr if p is None else p + pr
                p = p + pltpu.roll(p, 64, 1)
                p = p + pltpu.roll(p, 32, 1)
                if w > 0 and r0 < HALO:
                    pos = lax.broadcasted_iota(jnp.int32, (RB, 128), 0) + (base + r0)
                    p = jnp.where(pos >= DIL * w, p, -1e9)
                lg.append(p)
            mx = functools.reduce(jnp.maximum, lg)
            e = [jnp.exp2(l - mx) for l in lg]
            den = functools.reduce(lambda a, b: a + b, e)
            rinv = pltpu.reciprocal(den, approx=True)
            e = [ew * rinv for ew in e]
            os_ = []
            for t in range(NT):
                o = None
                for w in range(W):
                    ov = e[w] * kv_s[NT + t, pl.ds(b0 - DIL * w, RB), :]
                    o = ov if o is None else o + ov
                os_.append(o)
            return jnp.concatenate(os_, axis=1).astype(jnp.bfloat16)

        xu = xn_v[pl.ds(pl.multiple_of(base // 2, BM // 2), BM // 2), :]
        xn = pltpu.bitcast(xu, jnp.bfloat16)
        outs = [attention_piece(r0) for r0 in range(0, BM, RB)]
        keep = (xu[0:8, 0:128] | 1) != 0

        def lhs_for(pos):
            tied = [n for n in range(len(outs)) if 1 + n * (2 * NF - 1) // len(outs) == pos]
            if not tied:
                return xn
            head = xu[0:8, 0:128]
            for n in tied:
                head = jnp.where(keep, head, pltpu.bitcast(outs[n][0:16, 0:128], jnp.uint32))
            top = jnp.concatenate([head, xu[0:8, 128:]], axis=1)
            return pltpu.bitcast(jnp.concatenate([top, xu[8:]], axis=0), jnp.bfloat16)

        acc = None
        for c in range(NF):
            cs = slice(c * BF, (c + 1) * BF)
            g = jnp.dot(lhs_for(2 * c), wg_v[:, cs], preferred_element_type=jnp.float32)
            u = jnp.dot(lhs_for(2 * c + 1), wu_v[:, cs], preferred_element_type=jnp.float32)
            h = (_silu(g) * u).astype(jnp.bfloat16)
            d = jnp.dot(h, wd_v[cs, :], preferred_element_type=jnp.float32)
            acc = d if acc is None else acc + d
        o = jnp.concatenate(outs, axis=0)
        s = jnp.dot(o, pltpu.bitcast(wop_v[...], jnp.bfloat16), preferred_element_type=jnp.float32)
        gy = _silu(acc)
        cw = D // OSPLIT
        for j in range(OSPLIT):
            cols = slice(j * cw, (j + 1) * cw)
            out_v[rows, cols] = (in_v[rows, cols].astype(jnp.float32) + s[:, cols] * gy[:, cols]).astype(out_v.dtype)
            out_copy(i, j).start()
        return carry

    lax.fori_loop(0, NSTEP, main_body, 0)
    pltpu.make_async_copy(out_v, out_h, sem_out.at[0]).wait()


def _run(A_x, A_wqkv, A_wo, B_x, B_w_gate, B_w_up, B_w_down):
    del B_x
    hbm = pl.BlockSpec(memory_space=pl.ANY)
    out = pl.pallas_call(
        _kernel,
        in_specs=[hbm] * 6,
        out_specs=hbm,
        out_shape=jax.ShapeDtypeStruct((S, D), jnp.bfloat16),
        scratch_shapes=[
            pltpu.VMEM((S + 4 * D, D), jnp.bfloat16),
            pltpu.VMEM((S // 2, D), jnp.uint32),
            pltpu.VMEM((4, D // 2, D), jnp.uint32),
            pltpu.VMEM((D // 2, D), jnp.uint32),
            pltpu.VMEM((D, F), jnp.bfloat16),
            pltpu.VMEM((D, F), jnp.bfloat16),
            pltpu.VMEM((F, D), jnp.bfloat16),
            pltpu.VMEM((2 * NT, HALO + S, 128), jnp.float32),
            pltpu.VMEM((NT, S, 128), jnp.float32),
            pltpu.VMEM((2, S, 128), jnp.float32),
            pltpu.VMEM((8, D), jnp.float32),
            pltpu.VMEM((S, D), jnp.bfloat16),
            pltpu.SemaphoreType.DMA((NQM,)),
            pltpu.SemaphoreType.DMA((len(QSEG),)),
            pltpu.SemaphoreType.DMA((2 * NQM,)),
            pltpu.SemaphoreType.DMA((4,)),
            pltpu.SemaphoreType.DMA((1,)),
        ],
        compiler_params=pltpu.CompilerParams(vmem_limit_bytes=120 * 1024 * 1024),
    )(A_x.reshape(S, D), A_wqkv, A_wo, B_w_gate, B_w_up, B_w_down)
    return out.reshape(1, S, D)


@jax.jit
def pallas_recurrent_scan__sliding_local_dilated__swiglu_ffn__prompt_kernel(
    A_x: jax.Array,
    A_wqkv: jax.Array,
    A_wo: jax.Array,
    B_x: jax.Array,
    B_w_gate: jax.Array,
    B_w_up: jax.Array,
    B_w_down: jax.Array,
):
    return _run(A_x, A_wqkv, A_wo, B_x, B_w_gate, B_w_up, B_w_down)
```

```python
import functools

import numpy as np
import jax
import jax.numpy as jnp
import jax.experimental.pallas as pl
import jax.experimental.pallas.tpu as pltpu
from jax import lax

S, D, F = 2048, 1024, 3584
DH, W, DIL = 32, 8, 2
HALO = 16
NT = D // 128
LOG2E = 1.4426950408889634
QSCALE = DH ** -0.5 * LOG2E

BM = 256
BF = 512
RB = 16
QM = 512
QSEG = (384, 640)
QROWS, QCOLS = 128, 128
LNR = 16
QPR = 64
PR = 64
OSPLIT = 8

NSTEP = S // BM
NF = F // BF
NQM = S // QM
KC = D // NQM
WQ0 = S
WO0 = S + 3 * D


def _silu(x):
    return x * pltpu.reciprocal(1.0 + jnp.exp2(x * (-LOG2E)), approx=True)


def _swap_heads(xs):
    lane = lax.broadcasted_iota(jnp.int32, xs[0].shape, 1)
    g = lane >> 4
    e = lane & 15
    zs = []
    for s in range(NT):
        idx = (e & 3) * 32 + ((g - s) & 7) * 4 + (e >> 2)
        zs.append(jnp.take_along_axis(xs[s], idx, axis=1, mode="promise_in_bounds"))
    a = [zs[(-t) % NT] for t in range(NT)]
    for b in range(3):
        bit = ((g >> b) & 1) == 1
        a = [jnp.where(bit, a[(t - (1 << b)) % NT], a[t]) for t in range(NT)]
    out = []
    for t in range(NT):
        idx = ((((lane >> 2) & 7) + t) & 7) * 16 + (lane >> 5) * 4 + (lane & 3)
        out.append(jnp.take_along_axis(a[t], idx, axis=1, mode="promise_in_bounds"))
    return out


def _transpose_sublanes(xs):
    p = lax.broadcasted_iota(jnp.int32, xs[0].shape, 0)
    ys = [x if i == 0 else pltpu.roll(x, i, 0) for i, x in enumerate(xs)]
    a = [ys[(-t) % 8] for t in range(8)]
    for b in range(3):
        bit = ((p >> b) & 1) == 1
        a = [jnp.where(bit, a[(t - (1 << b)) % 8], a[t]) for t in range(8)]
    return [x if s == 0 else pltpu.roll(x, 8 - s, 0) for s, x in enumerate(a)]


def _tree_sum(xs):
    while len(xs) > 1:
        xs = [xs[2 * a] + xs[2 * a + 1] for a in range(len(xs) // 2)]
    return xs[0]


def _bf16_words(x):
    return pltpu.bitcast(x.astype(jnp.bfloat16), jnp.uint32)


def _kernel(x_h, wqkv_h, wo_h, wg_h, wu_h, wd_h, out_h,
            in_v, xn_v, wp_v, wop_v, wg_v, wu_v, wd_v, kv_s, q_s, st_s, cs_s, out_v,
            sem_x, sem_q, sem_kv, sem_w, sem_out):
    def x_copy(r):
        return pltpu.make_async_copy(x_h.at[pl.ds(r * QM, QM), :], in_v.at[pl.ds(r * QM, QM), :], sem_x.at[r])

    def wq_copy(i):
        c0 = sum(QSEG[:i])
        return pltpu.make_async_copy(wqkv_h.at[:, pl.ds(c0, QSEG[i])],
                                     in_v.at[pl.ds(WQ0, D), pl.ds(c0, QSEG[i])], sem_q.at[i])

    def wkv_copy(m, r):
        return pltpu.make_async_copy(wqkv_h.at[pl.ds(r * KC, KC), pl.ds(m * D, D)],
                                     in_v.at[pl.ds(WQ0 + m * D + r * KC, KC), :], sem_kv.at[(m - 1) * NQM + r])

    w_copies = [pltpu.make_async_copy(src, dst, sem_w.at[n])
                for n, (src, dst) in enumerate([(wg_h, wg_v), (wu_h, wu_v), (wd_h, wd_v)])]
    wo_copy = pltpu.make_async_copy(wo_h, in_v.at[pl.ds(WO0, D), :], sem_w.at[3])

    def out_copy(i, j):
        cw = D // OSPLIT
        return pltpu.make_async_copy(out_v.at[pl.ds(i * BM, BM), pl.ds(j * cw, cw)],
                                     out_h.at[pl.ds(i * BM, BM), pl.ds(j * cw, cw)], sem_out.at[0])

    def permute_weight_rows(ms, md, k0):
        for p0 in range(0, KC, 2 * PR):
            src = in_v[pl.ds(pl.multiple_of(WQ0 + ms * D + k0 + p0, 2 * PR), 2 * PR), :]
            u = pltpu.bitcast(src, jnp.uint32)
            ys = _swap_heads([u[:, s * 128:(s + 1) * 128] for s in range(NT)])
            dst0 = pl.multiple_of((k0 + p0) // 2, PR)
            for t in range(NT):
                wp_v[md, pl.ds(dst0, PR), t * 128:(t + 1) * 128] = ys[t]

    x_copy(0).start()
    for i in range(len(QSEG)):
        wq_copy(i).start()
    wkv_copy(1, 0).start()
    for r in range(1, NQM):
        x_copy(r).start()
        wkv_copy(1, r).start()
    for r in range(NQM):
        wkv_copy(2, r).start()
    wo_copy.start()
    kv_s[:, 0:HALO, :] = jnp.zeros((2 * NT, HALO, 128), jnp.float32)

    def layernorm_piece(r0):
        rows = pl.ds(pl.multiple_of(r0, LNR), LNR)
        x = in_v[rows, :].astype(jnp.float32)
        mu = jnp.mean(x, axis=-1, keepdims=True)
        xc = x - mu
        var = jnp.mean(xc * xc, axis=-1, keepdims=True)
        rs = lax.rsqrt(var + 1e-5)
        xn = _bf16_words(xc * rs)
        xn_v[pl.ds(pl.multiple_of(r0 // 2, LNR // 2), LNR // 2), :] = xn
        st_s[0, rows, :] = jnp.broadcast_to(mu, (LNR, 128))
        st_s[1, rows, :] = jnp.broadcast_to(rs * QSCALE, (LNR, 128))
        return xn

    def q_body(r, carry):
        r0 = pl.multiple_of(r * QM, QM)
        npc = QM // LNR
        for i, cw in enumerate(QSEG):
            last = i == len(QSEG) - 1
            c0 = sum(QSEG[:i])
            if i == 0:
                x_copy(r).wait()
            if last:
                wkv_copy(1, r).wait()

            @pl.when(r == 0)
            def _():
                wq_copy(i).wait()

            if last:
                @pl.when(r == 1)
                def _():
                    for cp in w_copies:
                        cp.start()

            keep = (pltpu.bitcast(in_v[pl.ds(r0, 16), 0:128], jnp.uint32) | 1) != 0
            subs = [(j, h) for j in range(cw // QCOLS) for h in range(QM // QROWS)]
            xbs = [in_v[pl.ds(pl.multiple_of(r0 + h * QROWS, QROWS), QROWS), :] for h in range(QM // QROWS)]
            mine = [n for n in range(npc) if c0 <= n * D // npc < c0 + cw]
            xns = {n: layernorm_piece(r0 + n * LNR) for n in mine}
            for k, (j, h) in enumerate(subs):
                lhs = xb = xbs[h]
                tied = [n for kk, n in enumerate(mine) if 2 + kk * (len(subs) + 2) // len(mine) == k]
                if tied:
                    head = pltpu.bitcast(xb[0:16, 0:128], jnp.uint32)
                    for n in tied:
                        head = jnp.where(keep, head, xns[n][0:8, 0:128])
                    top = jnp.concatenate([pltpu.bitcast(head, jnp.bfloat16), xb[0:16, 128:]], axis=1)
                    lhs = jnp.concatenate([top, xb[16:]], axis=0)
                cols = slice(c0 + j * QCOLS, c0 + (j + 1) * QCOLS)
                res = jnp.dot(lhs, in_v[WQ0:WQ0 + D, cols], preferred_element_type=jnp.float32)
                q_s[cols.start // 128, pl.ds(pl.multiple_of(r0 + h * QROWS, QROWS), QROWS), :] = res
            if last:
                ccols = pl.ds(pl.multiple_of(r * (D // NQM), D // NQM), D // NQM)
                cs = jnp.sum(in_v[WQ0:WQ0 + D, ccols].astype(jnp.float32), axis=0, keepdims=True)
                cs_s[:, ccols] = jnp.broadcast_to(cs, (8, D // NQM))
                permute_weight_rows(1, 1, r * KC)
        return carry

    lax.fori_loop(0, NQM, q_body, 0)

    QP = S // (2 * NQM)
    wo_copy.wait()

    def permute_wo_rows(t, res):
        cols = pl.ds(pl.multiple_of(t * 128, 128), 128)
        u = pltpu.bitcast(in_v[WO0:WO0 + D, cols], jnp.uint32)
        keep = (u[0:8] | 1) != 0
        for b in range(2):
            for dh in range(2):
                g = 2 * b + dh
                after = pltpu.bitcast(res[0:8, 2 * g * 128:(2 * g + 1) * 128], jnp.uint32)
                xa = [u[8 * (4 * (8 * b + i) + dh):8 * (4 * (8 * b + i) + dh) + 8] for i in range(8)]
                xc = [u[8 * (4 * (8 * b + i) + 2 + dh):8 * (4 * (8 * b + i) + 2 + dh) + 8] for i in range(8)]
                xa[0] = jnp.where(keep, xa[0], after)
                xc[0] = jnp.where(keep, xc[0], after)
                ta = _transpose_sublanes(xa)
                tc = _transpose_sublanes(xc)
                for s_ in range(8):
                    d2 = 8 * dh + s_
                    a, c = ta[s_], tc[s_]
                    wop_v[pl.ds(32 * d2 + 8 * b, 8), cols] = (a & 0xFFFF) | (c << 16)
                    wop_v[pl.ds(32 * d2 + 16 + 8 * b, 8), cols] = (a >> 16) | (c & np.uint32(0xFFFF0000))

    def kv_body(it, carry):
        m = 1 + it // NQM
        r = it % NQM

        @pl.when(m < 2)
        def _():
            wkv_copy(2, r).wait()

        r0 = pl.multiple_of(r * QM, QM)
        wmat = pltpu.bitcast(wp_v[m], jnp.bfloat16)
        xn = pltpu.bitcast(xn_v[pl.ds(pl.multiple_of(r0 // 2, QM // 2), QM // 2), :], jnp.bfloat16)
        res = jnp.dot(xn, wmat, preferred_element_type=jnp.float32)
        for t in range(NT):
            kv_s[(m - 1) * NT + t, pl.ds(r0 + HALO, QM), :] = res[:, t * 128:(t + 1) * 128]
        permute_weight_rows(2, m + 1, r * KC)
        permute_wo_rows(it, res)
        for p0 in range(0, QP, QPR):
            rows = pl.ds(pl.multiple_of(it * QP + p0, QPR), QPR)
            mu = st_s[0, rows, :]
            rs = st_s[1, rows, :]
            us = []
            for t in range(NT):
                cst = jnp.broadcast_to(cs_s[0:1, t * 128:(t + 1) * 128], (QPR, 128))
                us.append(_bf16_words((q_s[t, rows, :] - mu * cst) * rs))
            ys = _swap_heads(us)
            for t in range(NT):
                q_s[t, rows, :] = pltpu.bitcast(ys[t], jnp.bfloat16).astype(jnp.float32)
        return carry

    lax.fori_loop(0, 2 * NQM, kv_body, 0)

    for cp in w_copies:
        cp.wait()

    def main_body(i, carry):
        base = pl.multiple_of(i * BM, BM)
        rows = pl.ds(base, BM)

        def attention_piece(r0):
            b0 = base + (HALO + r0)
            q = [q_s[t, pl.ds(base + r0, RB), :] for t in range(NT)]
            lg = []
            for w in range(W):
                p = _tree_sum([q[t] * kv_s[t, pl.ds(b0 - DIL * w, RB), :] for t in range(NT)])
                p = p + pltpu.roll(p, 64, 1)
                p = p + pltpu.roll(p, 32, 1)
                if w > 0 and r0 < HALO:
                    pos = lax.broadcasted_iota(jnp.int32, (RB, 128), 0) + (base + r0)
                    p = jnp.where(pos >= DIL * w, p, -1e9)
                lg.append(p)
            mx = functools.reduce(jnp.maximum, lg)
            e = [jnp.exp2(l - mx) for l in lg]
            den = functools.reduce(lambda a, b: a + b, e)
            rinv = pltpu.reciprocal(den, approx=True)
            e = [ew * rinv for ew in e]
            os_ = [_tree_sum([e[w] * kv_s[NT + t, pl.ds(b0 - DIL * w, RB), :] for w in range(W)]) for t in range(NT)]
            return jnp.concatenate(os_, axis=1).astype(jnp.bfloat16)

        xu = xn_v[pl.ds(pl.multiple_of(base // 2, BM // 2), BM // 2), :]
        xn = pltpu.bitcast(xu, jnp.bfloat16)
        outs = [attention_piece(r0) for r0 in range(0, BM, RB)]
        keep = (xu[0:8, 0:128] | 1) != 0

        def lhs_for(pos):
            tied = [n for n in range(len(outs)) if 1 + n * (2 * NF - 1) // len(outs) == pos]
            if not tied:
                return xn
            head = xu[0:8, 0:128]
            for n in tied:
                head = jnp.where(keep, head, pltpu.bitcast(outs[n][0:16, 0:128], jnp.uint32))
            top = jnp.concatenate([head, xu[0:8, 128:]], axis=1)
            return pltpu.bitcast(jnp.concatenate([top, xu[8:]], axis=0), jnp.bfloat16)

        acc = None
        for c in range(NF):
            cs = slice(c * BF, (c + 1) * BF)
            g = jnp.dot(lhs_for(2 * c), wg_v[:, cs], preferred_element_type=jnp.float32)
            u = jnp.dot(lhs_for(2 * c + 1), wu_v[:, cs], preferred_element_type=jnp.float32)
            h = (_silu(g) * u).astype(jnp.bfloat16)
            d = jnp.dot(h, wd_v[cs, :], preferred_element_type=jnp.float32)
            acc = d if acc is None else acc + d
        o = jnp.concatenate(outs, axis=0)
        s = jnp.dot(o, pltpu.bitcast(wop_v[...], jnp.bfloat16), preferred_element_type=jnp.float32)
        gy = _silu(acc)
        cw = D // OSPLIT
        for j in range(OSPLIT):
            cols = slice(j * cw, (j + 1) * cw)
            out_v[rows, cols] = (in_v[rows, cols].astype(jnp.float32) + s[:, cols] * gy[:, cols]).astype(out_v.dtype)
            out_copy(i, j).start()
        return carry

    lax.fori_loop(0, NSTEP, main_body, 0)
    pltpu.make_async_copy(out_v, out_h, sem_out.at[0]).wait()


def _run(A_x, A_wqkv, A_wo, B_x, B_w_gate, B_w_up, B_w_down):
    del B_x
    hbm = pl.BlockSpec(memory_space=pl.ANY)
    out = pl.pallas_call(
        _kernel,
        in_specs=[hbm] * 6,
        out_specs=hbm,
        out_shape=jax.ShapeDtypeStruct((S, D), jnp.bfloat16),
        scratch_shapes=[
            pltpu.VMEM((S + 4 * D, D), jnp.bfloat16),
            pltpu.VMEM((S // 2, D), jnp.uint32),
            pltpu.VMEM((4, D // 2, D), jnp.uint32),
            pltpu.VMEM((D // 2, D), jnp.uint32),
            pltpu.VMEM((D, F), jnp.bfloat16),
            pltpu.VMEM((D, F), jnp.bfloat16),
            pltpu.VMEM((F, D), jnp.bfloat16),
            pltpu.VMEM((2 * NT, HALO + S, 128), jnp.float32),
            pltpu.VMEM((NT, S, 128), jnp.float32),
            pltpu.VMEM((2, S, 128), jnp.float32),
            pltpu.VMEM((8, D), jnp.float32),
            pltpu.VMEM((S, D), jnp.bfloat16),
            pltpu.SemaphoreType.DMA((NQM,)),
            pltpu.SemaphoreType.DMA((len(QSEG),)),
            pltpu.SemaphoreType.DMA((2 * NQM,)),
            pltpu.SemaphoreType.DMA((4,)),
            pltpu.SemaphoreType.DMA((1,)),
        ],
        compiler_params=pltpu.CompilerParams(vmem_limit_bytes=120 * 1024 * 1024),
    )(A_x.reshape(S, D), A_wqkv, A_wo, B_w_gate, B_w_up, B_w_down)
    return out.reshape(1, S, D)


@jax.jit
def pallas_recurrent_scan__sliding_local_dilated__swiglu_ffn__prompt_kernel(
    A_x: jax.Array,
    A_wqkv: jax.Array,
    A_wo: jax.Array,
    B_x: jax.Array,
    B_w_gate: jax.Array,
    B_w_up: jax.Array,
    B_w_down: jax.Array,
):
    return _run(A_x, A_wqkv, A_wo, B_x, B_w_gate, B_w_up, B_w_down)
```
